```python
import os as _os
_os.environ.setdefault('JAX_PLATFORMS', 'cpu')
import jax
import jax.numpy as jnp

def _softmax(x, axis=-1):
    return jax.nn.softmax(x, axis=axis)

def _gelu(x):
    return jax.nn.gelu(x, approximate=True)

def _silu(x):
    return jax.nn.silu(x)

def _sigmoid(x):
    return jax.nn.sigmoid(x)

def _layernorm(x, axis=-1, eps=1e-05):
    m = jnp.mean(x, axis=axis, keepdims=True)
    v = jnp.var(x, axis=axis, keepdims=True)
    return (x - m) / jnp.sqrt(v + eps)

def _scatter_add(tgt, idx, src, axis=0):
    return tgt.at[idx].add(src)

def _segment_sum(src, seg, n):
    return jax.ops.segment_sum(src, seg, n)

class _Rng:

    def __init__(self, key):
        self._k = key

    def _next(self):
        self._k, sub = jax.random.split(self._k)
        return sub

    def normal(self, shape):
        return jax.random.normal(self._next(), shape, dtype=jnp.bfloat16)

    def randint(self, lo, hi, shape):
        return jax.random.randint(self._next(), shape, lo, hi, dtype=jnp.int32)

    def uniform(self, shape, lo=0.0, hi=1.0):
        return jax.random.uniform(self._next(), shape, jnp.bfloat16, lo, hi)

    def permutation(self, n):
        return jax.random.permutation(self._next(), n)
kernel_name = 'interleave_layers__ssm_conv_h3__mixer_gmlp__prompt'

def setup_inputs():
    _rng = _Rng(jax.random.key(int.from_bytes(__import__("os").urandom(4), "little")))
    _w = lambda a: (lambda t: t.astype(jnp.bfloat16) if jnp.issubdtype(t.dtype, jnp.floating) else t)(jnp.asarray(a))

    def _A_setup():
        B, S, D = (1, 2048, 1024)
        ks = 4
        return {'q': _w((lambda *s: _rng.normal(s) * 0.05)(B, S, D)), 'k': _w((lambda *s: _rng.normal(s) * 1.6)(B, S, D)), 'v': _w((lambda *s: _rng.normal(s) * 1.6)(B, S, D)), 'shift_k': _w((lambda *s: _rng.normal(s) * 1.6)(D, ks) * 0.5), 'ssm_k': _w((lambda *s: _rng.normal(s) * 1.6)(D, S) * (1.0 / S ** 0.5)), 'ssm_D': _w((lambda *s: _rng.normal(s) * 1.6)(D))}
    _A_in = _A_setup()

    def _B_setup():
        B, S, D, F = (1, 2048, 1024, 3584)
        Fh = F // 2
        return {'x': _w((lambda *s: _rng.normal(s) * 0.05)(B, S, D)), 'w_in': _w((lambda *s: _rng.normal(s) * 0.8)(D, 2 * Fh)), 'w_sp': _w(0.01 * (lambda *s: _rng.normal(s) * 0.8)(S, S)), 'b_sp': _w(1.0 + 0.01 * (lambda *s: _rng.normal(s) * 0.2)(S)), 'w_out': _w((lambda *s: _rng.normal(s) * 0.2)(Fh, D))}
    _B_in = _B_setup()
    return {'A_q': _A_in['q'], 'A_k': _A_in['k'], 'A_v': _A_in['v'], 'A_shift_k': _A_in['shift_k'], 'A_ssm_k': _A_in['ssm_k'], 'A_ssm_D': _A_in['ssm_D'], 'B_x': _B_in['x'], 'B_w_in': _B_in['w_in'], 'B_w_sp': _B_in['w_sp'], 'B_b_sp': _B_in['b_sp'], 'B_w_out': _B_in['w_out']}

def reference(A_q, A_k, A_v, A_shift_k, A_ssm_k, A_ssm_D, B_x, B_w_in, B_w_sp, B_b_sp, B_w_out):

    def _A_ref(q, k, v, shift_k, ssm_k, ssm_D):
        B, S, D = q.shape
        ks = shift_k.shape[-1]
        k_pad = jnp.pad(k, ((0, 0), (ks - 1, 0), (0, 0)))
        k_shift = jnp.zeros_like(k)
        for t in range(ks):
            k_shift = k_shift + k_pad[:, t:t + S, :] * shift_k[:, ks - 1 - t][None, None, :]
        kv = k_shift * v
        L = 2 * S
        kv_pad = jnp.pad(kv, ((0, 0), (0, S), (0, 0)))
        kf_pad = jnp.pad(ssm_k, ((0, 0), (0, S)))
        kv_f = (lambda x, axes=(-2, -1): jnp.fft.rfft2(x.astype(jnp.float32), axes=axes))(kv_pad[:, None, :, :], axes=(1, 2))
        kf_f = (lambda x, axes=(-2, -1): jnp.fft.rfft2(x.astype(jnp.float32), axes=axes))(kf_pad[:, None, :], axes=(1, 2))
        kf_f = (lambda x, *d: x.transpose(*d))(kf_f, 1, 2, 0)
        y_f = kv_f * kf_f[None, :, :, :]
        y = (lambda x, s, axes=(-2, -1): jnp.fft.irfft2(x, s=s, axes=axes).astype(jnp.bfloat16))(y_f, (1, L), axes=(1, 2))[:, 0, :S, :]
        y = y + kv * ssm_D[None, None, :]
        return q * y

    def _B_ref(x, w_in, w_sp, b_sp, w_out):
        B, S, D = x.shape
        F = w_in.shape[-1]
        Fh = F // 2
        z = _gelu(jnp.einsum('bsd,df->bsf', x, w_in))
        z1 = z[..., :Fh].copy()
        z2 = _layernorm(z[..., Fh:], axis=-1)
        g = jnp.einsum('ts,bsf->btf', w_sp, z2) + b_sp[None, :, None]
        return jnp.einsum('bsf,fd->bsd', z1 * g, w_out)
    x = A_q
    x = x + _A_ref(_layernorm(x, axis=-1), A_k, A_v, A_shift_k, A_ssm_k, A_ssm_D)
    x = x + _B_ref(_layernorm(x, axis=-1), B_w_in, B_w_sp, B_b_sp, B_w_out)
    x = x + _A_ref(_layernorm(x, axis=-1), A_k, A_v, A_shift_k, A_ssm_k, A_ssm_D)
    x = x + _B_ref(_layernorm(x, axis=-1), B_w_in, B_w_sp, B_b_sp, B_w_out)
    return x
```

```python
import numpy as np
import jax
import jax.numpy as jnp
import jax.experimental.pallas as pl
import jax.experimental.pallas.tpu as pltpu

f32 = jnp.float32
bf16 = jnp.bfloat16
u32 = jnp.uint32

S = 2048
D = 1024
F = 3584
FH = F // 2
FQ = FH // 2
D2 = D // 2
C = 128
NC = S // C
NB = D // 128
TM = 256
H = TM // 2
NT = S // TM
EPS = 1e-5
KS = 4
TN = 256
WR = D2 // NB


def _dft_mats():
    f = np.arange(C, dtype=np.float64)
    b = np.arange(C, dtype=np.float64)
    perm = np.concatenate([np.concatenate([np.arange(8 * p, 8 * p + 8), C + np.arange(8 * p, 8 * p + 8)])
                           for p in range(C // 8)])
    fwds, invs = [], []
    for a in range(4):
        ang = 2.0 * np.pi * (f[:, None] + 0.5) * (b[None, :] + C * a) / (2 * C)
        fwd = np.concatenate([np.cos(ang), -np.sin(ang)], axis=0)
        inv = (fwd.T / C)[:, perm]
        fwds.append(fwd)
        invs.append(inv)
    return np.stack(fwds).astype(np.float32), np.stack(invs).astype(np.float32)


def _ln(x):
    m = jnp.mean(x, axis=-1, keepdims=True)
    xc = x - m
    v = jnp.mean(xc * xc, axis=-1, keepdims=True)
    return xc * jax.lax.rsqrt(v + EPS)


def _gelu(x):
    c0 = 0.7978845608028654
    inner = x * (c0 + (c0 * 0.044715) * (x * x))
    hx = 0.5 * x
    return hx + hx * jnp.tanh(inner)


def _dot(a, b):
    return jnp.dot(a, b, preferred_element_type=f32)


def _a_ops(a11, a12, a21, a22):
    return (a11 + a22, a21 + a22, a11, a22, a11 + a12, a21 - a11, a12 - a22)


def _b_ops(b11, b12, b21, b22):
    return (b11 + b22, b11, b12 - b22, b21 - b11, b22, b11 + b12, b21 + b22)


def _c_blocks(m):
    c11 = m[0] + m[3] - m[4] + m[6]
    c12 = m[2] + m[4]
    c21 = m[1] + m[3]
    c22 = m[0] - m[1] + m[2] + m[5]
    return c11, c12, c21, c22


def _chunks(n, w):
    out = []
    o = 0
    while o < n:
        e = min(n, o + w)
        out.append((o, e))
        o = e
    return out


def _toep(hv, uv, init, sign, order):
    hcache, ucache = {}, {}

    def gh(l):
        if l not in hcache:
            hcache[l] = hv(l)
        return hcache[l]

    def gu(l):
        if l not in ucache:
            ucache[l] = uv(l)
        return ucache[l]

    for g in range(0, len(order), 2):
        pair = (order[g], order[g + 1])
        acc = {a: (init[a] if init is not None else None) for a in pair}
        for j in range(max(pair) + 1):
            for a in pair:
                if j > a:
                    continue
                pr = gh(a - j) * gu(j)
                if acc[a] is None:
                    acc[a] = pr
                elif sign > 0:
                    acc[a] = acc[a] + pr
                else:
                    acc[a] = acc[a] - pr
        for a in pair:
            yield a, acc[a]


def _ld(ref, t, lo, hi):
    return pltpu.bitcast(ref[t, :, lo:hi], bf16)


def _st(ref, t, col0, row0, val):
    n, w = val.shape
    if isinstance(row0, int):
        rows = slice(row0 // 2, (row0 + n) // 2)
    else:
        rows = pl.ds(pl.multiple_of(row0 // 2, 8), n // 2)
    if isinstance(col0, int):
        cols = slice(col0, col0 + w)
    else:
        cols = pl.ds(pl.multiple_of(col0, 128), w)
    ref[t, rows, cols] = pltpu.bitcast(val, jnp.uint32)


def _kernel(zero_ref, q_hbm, k_hbm, v_hbm, sk_ref, h_hbm, dd_ref, win_hbm, wsp_hbm, bsp_ref, wout_hbm,
            fwd_ref, inv_ref,
            out_hbm,
            kbuf, vbuf, hbuf, qbuf, win_raw, win_s, wsp_raw, wout_raw, wout_s,
            ybuf, xa, xb, z1buf, z2ops, zs, a0, a1, ws0, pa, bcol, obuf,
            kf, spA, spB, wscA, wscB,
            sem_kvh, sem_win, sem_misc, sem_out):

    def kvh_copies(c):
        return (
            pltpu.make_async_copy(k_hbm.at[:, c * 128:(c + 1) * 128], kbuf.at[c], sem_kvh.at[c]),
            pltpu.make_async_copy(v_hbm.at[:, c * 128:(c + 1) * 128], vbuf.at[c], sem_kvh.at[c]),
            pltpu.make_async_copy(h_hbm.at[c], hbuf.at[c], sem_kvh.at[c]),
        )

    def win_copies(c):
        r = c * WR
        return (
            pltpu.make_async_copy(win_hbm.at[r:r + WR, :], win_raw.at[r:r + WR, :], sem_win.at[c]),
            pltpu.make_async_copy(win_hbm.at[D2 + r:D2 + r + WR, :], win_raw.at[D2 + r:D2 + r + WR, :],
                                  sem_win.at[c]),
        )

    QS = 2 * TM
    q_copy0 = pltpu.make_async_copy(q_hbm.at[0:QS, :], qbuf.at[0:QS, :], sem_misc.at[0])
    q_copy1 = pltpu.make_async_copy(q_hbm.at[QS:S, :], qbuf.at[QS:S, :], sem_misc.at[3])
    wout_copy = pltpu.make_async_copy(wout_hbm, wout_raw, sem_misc.at[1])
    wsp_copy = pltpu.make_async_copy(wsp_hbm, wsp_raw, sem_misc.at[2])

    def start_all(cps):
        for cp in cps:
            cp.start()

    def wait_all(cps):
        for cp in cps:
            cp.wait()

    start_all(kvh_copies(0))
    start_all(kvh_copies(1))
    start_all(win_copies(0))

    skf = sk_ref[...].astype(f32)
    ddf = dd_ref[...].astype(f32)
    for r in range(S // 128):
        row = bsp_ref[r:r + 1, :].astype(f32)
        bcol[r * 128:(r + 1) * 128, :] = jnp.broadcast_to(row, (128, 128)).T

    def win_presum(c, it):
        RG = 16
        r = pl.multiple_of(c * WR + (it // 2) * RG, RG)
        half = it % 2
        o = pl.multiple_of(half * FH, 128)
        b11 = win_raw[pl.ds(r, RG), pl.ds(o, FQ)].astype(f32)
        b12 = win_raw[pl.ds(r, RG), pl.ds(o + FQ, FQ)].astype(f32)
        b21 = win_raw[pl.ds(D2 + r, RG), pl.ds(o, FQ)].astype(f32)
        b22 = win_raw[pl.ds(D2 + r, RG), pl.ds(o + FQ, FQ)].astype(f32)
        ops = _b_ops(b11, b12, b21, b22)
        for t in range(7):
            _st(win_s, t, half * FQ, r, ops[t].astype(bf16))

    desc = list(range(NC - 1, -1, -1))
    asc = list(range(NC))

    def conv_stage(c):
        do_prod = 0 <= c < NB
        do_fwd = c + 1 < NB
        do_inv = c - 1 >= 0
        sp_cur, sp_nxt = (spA, spB) if c % 2 == 0 else (spB, spA)
        ws_cur, ws_prv = (wscA, wscB) if c % 2 == 0 else (wscB, wscA)
        if do_fwd:
            cn = c + 1
            w = [skf[t:t + 1, cn * 128:(cn + 1) * 128] for t in range(KS)]
            kf[0:8, :] = jnp.zeros((8, 128), f32)

        def body(it, carry):
            if do_inv:
                for e in range(2):
                    a = 2 * it + e
                    r = pl.multiple_of(a * C, C)
                    ybuf[c - 1, pl.ds(r, C), :] = _dot(inv_ref[a % 4], ws_prv[a])
            if do_fwd:
                r2 = pl.multiple_of(it * 2 * C, 2 * C)
                kf[8:8 + 2 * C, :] = kbuf[cn, pl.ds(r2, 2 * C), :].astype(f32)
                for e in range(2):
                    a = 2 * it + e
                    r = pl.multiple_of(a * C, C)
                    fwd = fwd_ref[a % 4]
                    hj = jax.lax.dot_general(fwd, hbuf[cn, :, pl.ds(r, C)],
                                             (((1,), (1,)), ((), ())), preferred_element_type=f32)
                    sp_nxt[2, a] = hj[:C]
                    sp_nxt[3, a] = hj[C:]
                    o = 8 + e * C
                    ks = w[0] * kf[o:o + C, :]
                    for t in range(1, KS):
                        ks = ks + w[t] * kf[o - t:o - t + C, :]
                    kv = (ks * vbuf[cn, pl.ds(r, C), :].astype(f32)).astype(bf16)
                    u = _dot(fwd, kv)
                    sp_nxt[0, a] = u[:C]
                    sp_nxt[1, a] = u[C:]
                kf[0:8, :] = kf[2 * C:2 * C + 8, :]
            if do_prod:
                for e in range(2):
                    p = 2 * it + e
                    rows = pl.ds(pl.multiple_of(p * 8, 8), 8)
                    ua = lambda l: sp_cur[0, l, rows, :]
                    ub = lambda l: sp_cur[1, l, rows, :]
                    hc = lambda l: sp_cur[2, l, rows, :]
                    hd = lambda l: sp_cur[3, l, rows, :]
                    k1 = dict(_toep(hc, lambda l: ua(l) + ub(l), None, 1, desc))
                    im = dict(_toep(lambda l: hd(l) - hc(l), ua, k1, 1, desc))
                    re = {}
                    orow = pl.ds(pl.multiple_of(p * 16, 16), 16)
                    for a, val in _toep(lambda l: hd(l) + hc(l), ub, k1, -1, asc):
                        re[a] = val
                        if a == 0:
                            wr, wi = re[0], im[0]
                        else:
                            wr, wi = re[a] + re[a - 1], im[a] + im[a - 1]
                        ws_cur[a, orow, :] = jnp.concatenate([wr, wi], axis=0).astype(bf16)
                win_presum(c, it)
            return carry

        jax.lax.fori_loop(0, NC // 2, body, 0)
        if do_fwd:
            sp_nxt[2, 0] = sp_nxt[2, 0] + ddf[cn:cn + 1, :]

    with jax.named_scope('conv'):
        for c in range(-1, NB + 1):
            if c + 3 < NB:
                start_all(kvh_copies(c + 3))
            if c + 2 < NB:
                start_all(win_copies(c + 2))
            if c == NB - 3:
                q_copy0.start()
            if c == NB - 2:
                q_copy1.start()
            if c == NB - 1:
                wout_copy.start()
                wsp_copy.start()
            if c + 1 < NB:
                wait_all(kvh_copies(c + 1))
            if 0 <= c < NB:
                wait_all(win_copies(c))
            conv_stage(c)

    q_copy0.wait()
    q_copy1.wait()

    def win_b(t, lo, hi):
        return _ld(win_s, t, lo, hi)

    def wout_b(t, lo, hi):
        return _ld(wout_s, t, lo, hi)

    RG = 16
    NG = H // RG

    def prologue_group(i, g, src, dst, a_ref):
        xn = []
        for hh in range(2):
            rows = pl.ds(pl.multiple_of(i * TM + hh * H + g * RG, RG), RG)
            x = src[rows, :].astype(f32)
            y = jnp.concatenate([ybuf[c, rows, :] for c in range(NB)], axis=1)
            x1 = x + _ln(x) * y
            dst[rows, :] = x1
            xn.append(_ln(x1))
        ops = _a_ops(xn[0][:, :D2], xn[0][:, D2:], xn[1][:, :D2], xn[1][:, D2:])
        for t in range(7):
            _st(a_ref, t, 0, g * RG, ops[t].astype(bf16))

    def z2_group(i, g):
        rq = pl.multiple_of(i * H + g * RG, RG)
        n1 = _ln(zs[g * RG:(g + 1) * RG, :])
        n2 = _ln(zs[H + g * RG:H + (g + 1) * RG, :])
        ops = _b_ops(n1[:, :FQ], n1[:, FQ:], n2[:, :FQ], n2[:, FQ:])
        for t in range(7):
            _st(z2ops, t, 0, rq, ops[t].astype(bf16))

    def mm1(i, a_ref, inext, src, dst, a_next):
        r = pl.multiple_of(i * TM, TM)
        z0 = zero_ref[0]

        def fence(ref, nrows, val):
            ref[pl.ds(pl.multiple_of(nrows + z0 * 16, 16), 16), 0:128] = val[0:16, 0:128].astype(ref.dtype)

        pend = list(range(NG))
        for (lo, hi) in _chunks(FQ, TN):
            m = []
            for t in range(7):
                m.append(_dot(_ld(a_ref, t, 0, D2), win_b(t, FQ + lo, FQ + hi)))
                if t in (0, 2, 4) and pend:
                    fence(src, S, m[-1])
                    prologue_group(inext, pend.pop(0), src, dst, a_next)
            c11, c12, c21, c22 = _c_blocks(m)
            zs[0:H, lo:hi] = _gelu(c11)
            zs[0:H, FQ + lo:FQ + hi] = _gelu(c12)
            zs[H:TM, lo:hi] = _gelu(c21)
            zs[H:TM, FQ + lo:FQ + hi] = _gelu(c22)
        pend = list(range(NG))
        for (lo, hi) in _chunks(FQ, TN):
            m = []
            for t in range(7):
                m.append(_dot(_ld(a_ref, t, 0, D2), win_b(t, lo, hi)))
                if t in (1, 3, 5) and pend:
                    fence(zs, TM, m[-1])
                    z2_group(i, pend.pop(0))
            c11, c12, c21, c22 = _c_blocks(m)
            z1buf[pl.ds(r, H), lo:hi] = _gelu(c11).astype(bf16)
            z1buf[pl.ds(r, H), FQ + lo:FQ + hi] = _gelu(c12).astype(bf16)
            z1buf[pl.ds(r + H, H), lo:hi] = _gelu(c21).astype(bf16)
            z1buf[pl.ds(r + H, H), FQ + lo:FQ + hi] = _gelu(c22).astype(bf16)

    def build_ws(i, ws_ref):
        G = 32
        for g in range(H // G):
            r1 = pl.ds(pl.multiple_of(i * TM + g * G, G), G)
            r2 = pl.ds(pl.multiple_of(i * TM + H + g * G, G), G)
            for t in range(NT):
                a11 = wsp_raw[r1, t * TM:t * TM + H]
                a12 = wsp_raw[r1, t * TM + H:(t + 1) * TM]
                a21 = wsp_raw[r2, t * TM:t * TM + H]
                a22 = wsp_raw[r2, t * TM + H:(t + 1) * TM]
                ops = _a_ops(a11.astype(f32), a12.astype(f32), a21.astype(f32), a22.astype(f32))
                for u in range(7):
                    if u == 2:
                        val = a11
                    elif u == 3:
                        val = a22
                    else:
                        val = ops[u].astype(bf16)
                    _st(ws_ref, u, t * H, g * G, val)

    def mm23(i, ws_ref, src, store):
        r = pl.multiple_of(i * TM, TM)
        for (lo, hi) in _chunks(FQ, TN):
            wdt = hi - lo
            m = [_dot(_ld(ws_ref, t, 0, S // 2), _ld(z2ops, t, lo, hi)) for t in range(7)]
            c11, c12, c21, c22 = _c_blocks(m)
            b1 = jnp.concatenate([bcol[pl.ds(r, H), :]] * (wdt // 128), axis=1)
            b2 = jnp.concatenate([bcol[pl.ds(r + H, H), :]] * (wdt // 128), axis=1)
            p11 = z1buf[pl.ds(r, H), lo:hi].astype(f32) * (c11 + b1)
            p12 = z1buf[pl.ds(r, H), FQ + lo:FQ + hi].astype(f32) * (c12 + b1)
            p21 = z1buf[pl.ds(r + H, H), lo:hi].astype(f32) * (c21 + b2)
            p22 = z1buf[pl.ds(r + H, H), FQ + lo:FQ + hi].astype(f32) * (c22 + b2)
            ops = _a_ops(p11, p12, p21, p22)
            for t in range(7):
                _st(pa, t, lo, 0, ops[t].astype(bf16))
        build_ws(jnp.minimum(i + 1, NT - 1), ws_ref)
        for (lo, hi) in _chunks(D2, TN):
            m = [_dot(_ld(pa, t, 0, FQ), wout_b(t, lo, hi)) for t in range(7)]
            c11, c12, c21, c22 = _c_blocks(m)
            store(0, lo, hi, src[pl.ds(r, H), lo:hi] + c11)
            store(0, D2 + lo, D2 + hi, src[pl.ds(r, H), D2 + lo:D2 + hi] + c12)
            store(1, lo, hi, src[pl.ds(r + H, H), lo:hi] + c21)
            store(1, D2 + lo, D2 + hi, src[pl.ds(r + H, H), D2 + lo:D2 + hi] + c22)

    def out_copy(i, slot):
        r = pl.multiple_of(i * TM, TM)
        return pltpu.make_async_copy(obuf.at[slot], out_hbm.at[pl.ds(r, TM), :], sem_out.at[slot])

    for layer in range(2):
        src = qbuf if layer == 0 else xa
        dst = xa if layer == 0 else xb

        for g in range(NG):
            prologue_group(0, g, src, dst, a0)

        def p1_body(ii, carry, src=src, dst=dst):
            i = 2 * ii
            mm1(i, a0, i + 1, src, dst, a1)
            mm1(i + 1, a1, jnp.minimum(i + 2, NT - 1), src, dst, a0)
            return carry

        with jax.named_scope(f'p1_{layer}'):
            jax.lax.fori_loop(0, NT // 2, p1_body, 0)

        if layer == 0:
            wout_copy.wait()
            wsp_copy.wait()
            RB = 64

            def wout_presum(g, carry):
                r = pl.multiple_of(g * RB, RB)
                b11 = wout_raw[pl.ds(r, RB), 0:D2].astype(f32)
                b12 = wout_raw[pl.ds(r, RB), D2:D].astype(f32)
                b21 = wout_raw[pl.ds(FQ + r, RB), 0:D2].astype(f32)
                b22 = wout_raw[pl.ds(FQ + r, RB), D2:D].astype(f32)
                ops = _b_ops(b11, b12, b21, b22)
                for t in range(7):
                    _st(wout_s, t, 0, r, ops[t].astype(bf16))
                return carry
            with jax.named_scope('wout_presum'):
                jax.lax.fori_loop(0, FQ // RB, wout_presum, 0)

        build_ws(0, ws0)

        if layer == 0:
            def p2_body(i, carry):
                r = pl.multiple_of(i * TM, TM)

                def store(hh, lo, hi, val):
                    xa[pl.ds(r + hh * H, H), lo:hi] = val
                mm23(i, ws0, xa, store)
                return carry
            with jax.named_scope(f'p2_{layer}'):
                jax.lax.fori_loop(0, NT, p2_body, 0)
        else:
            def p2_body(i, carry):
                slot = i % 2

                def store(hh, lo, hi, val):
                    obuf[slot, hh * H:(hh + 1) * H, lo:hi] = val.astype(bf16)

                @pl.when(i >= 2)
                def _():
                    out_copy(i - 2, slot).wait()
                mm23(i, ws0, xb, store)
                out_copy(i, slot).start()
                return carry
            with jax.named_scope(f'p2_{layer}'):
                jax.lax.fori_loop(0, NT, p2_body, 0)
            out_copy(NT - 2, 0).wait()
            out_copy(NT - 1, 1).wait()


@jax.jit
def pallas_interleave_layers__ssm_conv_h3__mixer_gmlp__prompt_kernel(
    A_q: jax.Array,
    A_k: jax.Array,
    A_v: jax.Array,
    A_shift_k: jax.Array,
    A_ssm_k: jax.Array,
    A_ssm_D: jax.Array,
    B_x: jax.Array,
    B_w_in: jax.Array,
    B_w_sp: jax.Array,
    B_b_sp: jax.Array,
    B_w_out: jax.Array,
):
    fwd_np, inv_np = _dft_mats()
    fwd = jnp.asarray(fwd_np, dtype=bf16)
    inv = jnp.asarray(inv_np, dtype=bf16)
    zero = jnp.zeros((1,), jnp.int32)

    any_spec = pl.BlockSpec(memory_space=pl.ANY)
    vmem_spec = pl.BlockSpec(memory_space=pltpu.VMEM)
    smem_spec = pl.BlockSpec(memory_space=pltpu.SMEM)

    scratch = [
        pltpu.VMEM((NB, S, 128), bf16),
        pltpu.VMEM((NB, S, 128), bf16),
        pltpu.VMEM((NB, 128, S), bf16),
        pltpu.VMEM((S + 16, D), bf16),
        pltpu.VMEM((D, F), bf16),
        pltpu.VMEM((7, D2 // 2, FH), u32),
        pltpu.VMEM((S, S), bf16),
        pltpu.VMEM((FH, D), bf16),
        pltpu.VMEM((7, FQ // 2, D2), u32),
        pltpu.VMEM((NB, S, 128), f32),
        pltpu.VMEM((S + 16, D), f32),
        pltpu.VMEM((S, D), f32),
        pltpu.VMEM((S, FH), bf16),
        pltpu.VMEM((7, S // 4, FQ), u32),
        pltpu.VMEM((TM + 16, FH), f32),
        pltpu.VMEM((7, H // 2, D2), u32),
        pltpu.VMEM((7, H // 2, D2), u32),
        pltpu.VMEM((7, H // 2, S // 2), u32),
        pltpu.VMEM((7, H // 2, FQ), u32),
        pltpu.VMEM((S, 128), f32),
        pltpu.VMEM((2, TM, D), bf16),
        pltpu.VMEM((2 * C + 8, 128), f32),
        pltpu.VMEM((4, NC, C, 128), f32),
        pltpu.VMEM((4, NC, C, 128), f32),
        pltpu.VMEM((NC, 2 * C, 128), bf16),
        pltpu.VMEM((NC, 2 * C, 128), bf16),
        pltpu.SemaphoreType.DMA((NB,)),
        pltpu.SemaphoreType.DMA((NB,)),
        pltpu.SemaphoreType.DMA((4,)),
        pltpu.SemaphoreType.DMA((2,)),
    ]

    out = pl.pallas_call(
        _kernel,
        in_specs=[smem_spec, any_spec, any_spec, any_spec, vmem_spec, any_spec, vmem_spec,
                  any_spec, any_spec, vmem_spec, any_spec, vmem_spec, vmem_spec],
        out_specs=any_spec,
        out_shape=jax.ShapeDtypeStruct((S, D), bf16),
        scratch_shapes=scratch,
        compiler_params=pltpu.CompilerParams(vmem_limit_bytes=127 * 1024 * 1024),
    )(
        zero,
        A_q.reshape(S, D), A_k.reshape(S, D), A_v.reshape(S, D),
        A_shift_k.T, A_ssm_k.reshape(NB, 128, S), A_ssm_D.reshape(NB, 128),
        B_w_in, B_w_sp, B_b_sp.reshape(S // 128, 128), B_w_out,
        fwd, inv,
    )
    return out.reshape(1, S, D)
```

```python
import numpy as np
import jax
import jax.numpy as jnp
import jax.experimental.pallas as pl
import jax.experimental.pallas.tpu as pltpu

f32 = jnp.float32
bf16 = jnp.bfloat16
u32 = jnp.uint32

S = 2048
D = 1024
F = 3584
FH = F // 2
FQ = FH // 2
D2 = D // 2
C = 128
NC = S // C
NB = D // 128
TM = 256
H = TM // 2
NT = S // TM
EPS = 1e-5
KS = 4
TN = 256
WR = D2 // NB
PG = 4
CP = C + 8
LEAD = 3
STR = 1.0
PMODE = 1
ZK = 3
PW = 256
ZW = 256
PA = (5, 48)
ZA = (7, 48)


def _pack_rows(m):
    b = m.astype(bf16).view(np.uint16).astype(np.uint32)
    return b[0::2] | (b[1::2] << 16)


def _dft_mats():
    f = np.arange(C, dtype=np.float64)
    b = np.arange(C, dtype=np.float64)
    perm_f = np.concatenate([np.concatenate([np.arange(8 * p, 8 * p + 8), C + np.arange(8 * p, 8 * p + 8)])
                             for p in range(C // 8)])
    perm_i = np.stack([np.arange(C), C + np.arange(C)], axis=1).reshape(-1)
    fwds, invs = [], []
    for a in range(4):
        ang = 2.0 * np.pi * (f[:, None] + 0.5) * (b[None, :] + C * a) / (2 * C)
        fwd = np.concatenate([np.cos(ang), -np.sin(ang)], axis=0)
        inv = (fwd.T / C)[:, perm_i]
        fwds.append(_pack_rows(fwd[perm_f].astype(np.float32)))
        invs.append(_pack_rows(inv.astype(np.float32)))
    return np.stack(fwds), np.stack(invs)


def _ln(x):
    m = jnp.mean(x, axis=-1, keepdims=True)
    xc = x - m
    v = jnp.mean(xc * xc, axis=-1, keepdims=True)
    return xc * jax.lax.rsqrt(v + EPS)


def _gelu(x):
    c0 = 0.7978845608028654
    inner = x * (c0 + (c0 * 0.044715) * (x * x))
    hx = 0.5 * x
    return hx + hx * jnp.tanh(inner)


def _dot(a, b):
    return jnp.dot(a, b, preferred_element_type=f32)


def _a_ops(a11, a12, a21, a22):
    return (a11 + a22, a21 + a22, a11, a22, a11 + a12, a21 - a11, a12 - a22)


def _b_ops(b11, b12, b21, b22):
    return (b11 + b22, b11, b12 - b22, b21 - b11, b22, b11 + b12, b21 + b22)


def _c_blocks(m):
    c11 = m[0] + m[3] - m[4] + m[6]
    c12 = m[2] + m[4]
    c21 = m[1] + m[3]
    c22 = m[0] - m[1] + m[2] + m[5]
    return c11, c12, c21, c22


def _chunks(n, w):
    out = []
    o = 0
    while o < n:
        e = min(n, o + w)
        out.append((o, e))
        o = e
    return out


def _gate(x, dep):
    if dep is None:
        return x
    if x.shape[0] == 8:
        return x | dep
    return jnp.concatenate([x[0:8] | dep, x[8:]], axis=0)


def _ld(ref, t, lo, hi):
    return pltpu.bitcast(ref[t, :, lo:hi], bf16)


def _st(ref, t, col0, row0, val):
    n, w = val.shape
    if isinstance(row0, int):
        rows = slice(row0 // 2, (row0 + n) // 2)
    else:
        rows = pl.ds(pl.multiple_of(row0 // 2, 8), n // 2)
    if isinstance(col0, int):
        cols = slice(col0, col0 + w)
    else:
        cols = pl.ds(pl.multiple_of(col0, 128), w)
    pk = pltpu.bitcast(val, jnp.uint32)
    ref[t, rows, cols] = pk
    return pk


def _pk(e, o):
    return pltpu.bitcast(pltpu.pack_elementwise([e, o], packed_dtype=bf16), u32)


def _unpk(u, idx):
    return pltpu.unpack_elementwise(u, index=idx, packed_dtype=bf16, unpacked_dtype=f32)


def _ld_eo(ref, r, c0, c1):
    return jnp.concatenate(
        [jnp.concatenate([ref[c, pl.ds(r, 8, stride=2), :], ref[c, pl.ds(r + 1, 8, stride=2), :]], axis=0)
         for c in range(c0, c1)], axis=1)


def _st_eo(ref, t, col0, row0, val):
    pk = _pk(val[0:8], val[8:16])
    rows = slice(row0 // 2, row0 // 2 + 8) if isinstance(row0, int) else pl.ds(pl.multiple_of(row0 // 2, 8), 8)
    ref[t, rows, col0:col0 + val.shape[1]] = pk
    return pk


def _or_all(vals):
    parts = []
    for v in vals:
        for r in range(0, v.shape[0], 8):
            for c in range(0, v.shape[1], 128):
                parts.append(v[r:r + 8, c:c + 128])
    while len(parts) > 1:
        parts = [parts[i] | parts[i + 1] if i + 1 < len(parts) else parts[i] for i in range(0, len(parts), 2)]
    return parts[0]


def _ldg(ref, t, lo, hi, deps):
    w = ref[t, :, lo:hi]
    if any(d is not None for d in deps):
        top = [w[0:8, j * 128:(j + 1) * 128] if d is None else w[0:8, j * 128:(j + 1) * 128] | d
               for j, d in enumerate(deps)]
        top = top[0] if len(top) == 1 else jnp.concatenate(top, axis=1)
        w = jnp.concatenate([top, w[8:]], axis=0)
    return pltpu.bitcast(w, bf16)


def _stat_dep(x):
    b = pltpu.bitcast(jnp.broadcast_to(x, (16, 128)), u32)
    return b[0:8] | b[8:16]


def _kernel(zero_ref, q_hbm, k_hbm, v_hbm, sk_hbm, h_hbm, dd_hbm, win_hbm, wsp_hbm, bsp_hbm, wout_hbm,
            fwd_hbm, inv_hbm, sel_hbm,
            out_hbm,
            kbuf, vbuf, hbuf, qbuf, win_raw, win_s, wsp_raw, wout_raw, wout_s,
            ybuf, xa, xb, z1buf, z2ops, zs, a0, a1, ws0, pa, bcol, obuf,
            kf, spA, spB, wscA, wscB, cpar,
            sk_ref, dd_ref, bsp_ref, fwd_ref, inv_ref, sel_ref,
            sem_kvh, sem_win, sem_misc, sem_out, sem_q0, sem_small):

    def kvh_copies(c):
        cols = pl.ds(pl.multiple_of(c * 128, 128), 128)
        return (
            pltpu.make_async_copy(k_hbm.at[:, cols], kbuf.at[c], sem_kvh.at[c]),
            pltpu.make_async_copy(v_hbm.at[:, cols], vbuf.at[c], sem_kvh.at[c]),
            pltpu.make_async_copy(h_hbm.at[c], hbuf.at[c], sem_kvh.at[c]),
        )

    def win_copies(c):
        r1 = pl.ds(pl.multiple_of(c * WR, WR), WR)
        r2 = pl.ds(pl.multiple_of(D2 + c * WR, WR), WR)
        return (
            pltpu.make_async_copy(win_hbm.at[r1, :], win_raw.at[r1, :], sem_win.at[c]),
            pltpu.make_async_copy(win_hbm.at[r2, :], win_raw.at[r2, :], sem_win.at[c]),
        )

    QS = 3 * TM
    q_copy0 = pltpu.make_async_copy(q_hbm.at[0:QS, :], qbuf.at[0:QS, :], sem_misc.at[0])
    q_copy1 = pltpu.make_async_copy(q_hbm.at[QS:S, :], qbuf.at[QS:S, :], sem_misc.at[3])
    wout_copy = pltpu.make_async_copy(wout_hbm, wout_raw, sem_misc.at[1])
    wsp_copy = pltpu.make_async_copy(wsp_hbm, wsp_raw, sem_misc.at[2])

    def start_all(cps):
        for cp in cps:
            cp.start()

    def wait_all(cps):
        for cp in cps:
            cp.wait()

    def kvh0_copies(it):
        rows = pl.ds(pl.multiple_of(it * (S // 4), S // 4), S // 4)
        return (
            pltpu.make_async_copy(k_hbm.at[rows, 0:128], kbuf.at[0, rows, :], sem_q0.at[it]),
            pltpu.make_async_copy(v_hbm.at[rows, 0:128], vbuf.at[0, rows, :], sem_q0.at[it]),
            pltpu.make_async_copy(h_hbm.at[0, :, rows], hbuf.at[0, :, rows], sem_q0.at[it]),
        )

    small0 = (
        pltpu.make_async_copy(sk_hbm, sk_ref, sem_small.at[0]),
        pltpu.make_async_copy(dd_hbm, dd_ref, sem_small.at[0]),
        pltpu.make_async_copy(bsp_hbm, bsp_ref, sem_small.at[0]),
    )
    fwd_copy = pltpu.make_async_copy(fwd_hbm, fwd_ref, sem_small.at[1])
    small2 = (
        pltpu.make_async_copy(inv_hbm, inv_ref, sem_small.at[2]),
        pltpu.make_async_copy(sel_hbm, sel_ref, sem_small.at[2]),
    )

    start_all(small0)
    fwd_copy.start()
    start_all(kvh0_copies(0))
    wscB[...] = jnp.zeros(wscB.shape, u32)
    wait_all(small0)
    fwd_copy.wait()
    for it in range(1, 4):
        start_all(kvh0_copies(it))
    start_all(small2)

    skf = sk_ref[...].astype(f32)
    ddf = dd_ref[...].astype(f32)
    for c in range(NB):
        cpar[c, 0:KS, :] = skf[:, c * 128:(c + 1) * 128]
        cpar[c, KS:KS + 1, :] = ddf[c:c + 1, :]
    for r in range(S // 128):
        row = bsp_ref[r:r + 1, :].astype(f32)
        bcol[r * 128:(r + 1) * 128, :] = jnp.broadcast_to(row, (128, 128)).T

    def win_presum(c, it, dep):
        RG = 32
        g, half, cb = it // 14, (it // 7) % 2, it % 7
        r = pl.multiple_of(c * WR + g * RG, RG)
        r2 = pl.multiple_of(D2 + c * WR + g * RG, RG)
        o = half * FH + cb * 128
        b11 = pltpu.bitcast(win_raw[pl.ds(r, RG), o:o + 128], u32)
        b12 = pltpu.bitcast(win_raw[pl.ds(r, RG), o + FQ:o + FQ + 128], u32)
        b21 = pltpu.bitcast(win_raw[pl.ds(r2, RG), o:o + 128], u32)
        b22 = pltpu.bitcast(win_raw[pl.ds(r2, RG), o + FQ:o + FQ + 128], u32)
        rhs = jnp.concatenate([_gate(b11, dep), b12, b21, b22], axis=0)
        sums = _dot(pltpu.bitcast(sel_ref[...], bf16), pltpu.bitcast(rhs, bf16))
        col = half * FQ + cb * 128
        for k, t in enumerate((0, 2, 3, 5, 6)):
            for hh in range(2):
                _st_eo(win_s, t, col, r + 16 * hh, sums[k * RG + 16 * hh:k * RG + 16 * hh + 16])
        _st(win_s, 1, col, r, pltpu.bitcast(b11, bf16))
        _st(win_s, 4, col, r, pltpu.bitcast(b22, bf16))

    zsc = [zero_ref[g] for g in range(NC // PG)]
    zmask = jnp.full((8, 128), zsc[0], jnp.int32).astype(u32)

    def conv_stage(c, par, do_prod, do_fwd, do_inv, chunks=range(NC), a0=0):
        sp_cur, sp_nxt = (spA, spB) if par == 0 else (spB, spA)
        ws_cur, ws_prv = (wscA, wscB) if par == 0 else (wscB, wscA)
        if isinstance(c, int):
            cn, cp = c + 1, c - 1
        else:
            cn = jnp.minimum(c + 1, NB - 1)
            cp = jnp.where(c == 0, NB - 1, c - 1)

        def crow(a, off=0):
            if isinstance(a0, int):
                return slice((a0 + a) * C + off, (a0 + a + 1) * C + off)
            return pl.ds(pl.multiple_of(a0 * C, C) + (a * C + off), C)

        def inv(a, dep):
            wv = ws_prv[a0 + a]
            wv = jnp.concatenate([_gate(wv[:C // 2], dep), _gate(wv[C // 2:], dep)], axis=0)
            ybuf[cp, crow(a), :] = _dot(pltpu.bitcast(inv_ref[a % 4], bf16), pltpu.bitcast(wv, bf16))

        def hf(a, dep):
            hv = hbuf[cn, :, crow(a)]
            if dep is not None:
                hv = pltpu.bitcast(_gate(pltpu.bitcast(hv, u32), dep), bf16)
            hj = jax.lax.dot_general(pltpu.bitcast(fwd_ref[a % 4], bf16), hv,
                                     (((1,), (1,)), ((), ())), preferred_element_type=f32)
            if a == 0:
                dd = cpar[cn, KS:KS + 1, :]
                if not isinstance(a0, int):
                    dd = jnp.where(a0 == 0, dd, 0.0)
            for p in range(C // 8):
                re = hj[16 * p:16 * p + 8]
                im = hj[16 * p + 8:16 * p + 16]
                if a == 0:
                    re = re + dd
                sp_nxt[3, a0 + a, 8 * p:8 * p + 8, :] = re
                sp_nxt[4, a0 + a, 8 * p:8 * p + 8, :] = im - re
                sp_nxt[5, a0 + a, 8 * p:8 * p + 8, :] = im + re

        def uf(a, dep):
            w = [cpar[cn, t:t + 1, :] for t in range(KS)]
            kf[crow(a, 8), :] = kbuf[cn, crow(a), :].astype(f32)
            ks = w[0] * kf[crow(a, 8), :]
            for t in range(1, KS):
                ks = ks + w[t] * kf[crow(a, 8 - t), :]
            kvf = ks * vbuf[cn, crow(a), :].astype(f32)
            if dep is not None:
                kvf = pltpu.bitcast(_gate(pltpu.bitcast(kvf, u32), dep), f32)
            u = _dot(pltpu.bitcast(fwd_ref[a % 4], bf16), kvf.astype(bf16))
            for p in range(C // 8):
                re = u[16 * p:16 * p + 8]
                im = u[16 * p + 8:16 * p + 16]
                sp_nxt[0, a0 + a, 8 * p:8 * p + 8, :] = im + re
                sp_nxt[1, a0 + a, 8 * p:8 * p + 8, :] = re
                sp_nxt[2, a0 + a, 8 * p:8 * p + 8, :] = im

        prev = {}

        def pgroup(p, g, dep):
            rows = pl.ds(pl.multiple_of(p * 8 + zsc[g] * 8, 8), 8)
            outs = range(g * PG, (g + 1) * PG)
            acc, hw = {}, {}
            for j in range((g + 1) * PG):
                uu = [sp_cur[k, j, rows, :] for k in range(3)]
                if j == 0 and dep is not None:
                    uu = [pltpu.bitcast(_gate(pltpu.bitcast(x, u32), dep), f32) for x in uu]
                for a in outs:
                    l = a - j
                    if l < 0:
                        continue
                    if l not in hw:
                        hw[l] = [sp_cur[3 + k, l, rows, :] for k in range(3)]
                    for k in range(3):
                        pr = hw[l][k] * uu[k]
                        acc[a, k] = pr if (a, k) not in acc else acc[a, k] + pr
            d = None
            for a in outs:
                re = acc[a, 0] - acc[a, 2]
                im = acc[a, 0] + acc[a, 1]
                if a == 0:
                    wr, wi = re, im
                else:
                    wr, wi = re + prev['re'], im + prev['im']
                prev['re'], prev['im'] = re, im
                pk = pltpu.bitcast(pltpu.pack_elementwise([wr, wi], packed_dtype=bf16), u32)
                ws_cur[a, p * 8:p * 8 + 8, :] = pk
                if a % 2 == 1:
                    d = pk if d is None else d | pk
            return d & zmask

        dots = []
        for a in chunks:
            if do_fwd:
                dots += [(uf, a), (hf, a)]
            if do_inv:
                dots += [(inv, a)]
            if do_inv and PMODE == 0:
                dots += [(lambda it, dep: win_presum(cp, it, dep), it) for it in range(a * 28 // NC, (a + 1) * 28 // NC)]
        if do_inv and PMODE == 1:
            dots += [(lambda it, dep: win_presum(cp, it, dep), it) for it in range(28)]
        cost = [160 if fn not in (uf, hf, inv) else 256 for fn, _ in dots]
        pos = (np.cumsum(cost) - cost - LEAD * 256) / sum(cost) * STR
        nd = len(dots)
        if not do_prod:
            for fn, a in dots:
                fn(a, None)
            return
        ng = NC // PG
        wts = [sum(a + 1 for a in range(g * PG, (g + 1) * PG)) for g in range(ng)] * (C // 8)
        cum = np.cumsum(wts) / sum(wts)
        d = 0
        while d < nd and pos[d] <= 0:
            dots[d][0](dots[d][1], None)
            d += 1
        dep = None
        i = 0
        for p in range(C // 8):
            for g in range(ng):
                dep = pgroup(p, g, dep)
                while d < nd and pos[d] <= cum[i]:
                    dots[d][0](dots[d][1], dep)
                    d += 1
                i += 1

    kf[0:8, :] = jnp.zeros((8, 128), f32)

    with jax.named_scope('conv'):
        start_all(kvh_copies(1))

        def first_body(it, carry):
            wait_all(kvh0_copies(it))
            conv_stage(-1, 1, False, True, False, range(4), it * 4)
            return carry
        jax.lax.fori_loop(0, NC // 4, first_body, 0)
        wait_all(small2)

        def conv_body(ii, carry):
            for e in range(2):
                c = 2 * ii + e

                if e == 0:
                    wait_all(kvh_copies(c + 1))

                    @pl.when(c > 0)
                    def _():
                        wait_all(win_copies(c - 1))

                    @pl.when(c + 2 < NB)
                    def _():
                        start_all(kvh_copies(c + 2))

                    @pl.when(c + 2 == NB)
                    def _():
                        q_copy0.start()
                else:
                    wait_all(win_copies(c - 1))

                    @pl.when(c + 1 < NB)
                    def _():
                        wait_all(kvh_copies(c + 1))
                        start_all(kvh_copies(c + 2))
                start_all(win_copies(c))
                conv_stage(c, e, True, True, True)
            return carry
        jax.lax.fori_loop(0, NB // 2, conv_body, 0)

    q_copy0.wait()
    wait_all(win_copies(NB - 1))
    q_copy1.start()
    conv_stage(NB, 0, False, False, True)

    def win_b(t, lo, hi):
        return _ld(win_s, t, lo, hi)

    def wout_b(t, lo, hi):
        return _ld(wout_s, t, lo, hi)

    RG = 16
    NG = H // RG

    def prologue_steps(i, src, dst, a_ref):
        for g in range(NG):
            st = []
            for hh in range(2):
                r = pl.multiple_of(i * TM + hh * H + g * RG, RG)
                if src is qbuf:
                    xq = pltpu.bitcast(src[pl.ds(r, RG), :], u32)
                    x = jnp.concatenate([_unpk(xq, 0), _unpk(xq, 1)], axis=0)
                else:
                    x = _ld_eo(src, r, 0, NB)
                x1 = x + _ln(x) * _ld_eo(ybuf, r, 0, NB)
                for c in range(NB):
                    dst[c, pl.ds(r, 8, stride=2), :] = x1[0:8, c * 128:(c + 1) * 128]
                    dst[c, pl.ds(r + 1, 8, stride=2), :] = x1[8:16, c * 128:(c + 1) * 128]
                m = jnp.mean(x1, axis=-1, keepdims=True)
                xc = x1 - m
                rs = jax.lax.rsqrt(jnp.mean(xc * xc, axis=-1, keepdims=True) + EPS)
                st.append((pl.multiple_of(i * TM + hh * H + g * RG + zsc[1] * RG, RG), m, rs))
                yield _stat_dep(rs) & zmask
            for (lo, hi) in _chunks(D2, PW):
                q4 = []
                for hh in range(2):
                    rw, m, rs = st[hh]
                    for o in (0, D2):
                        q4.append((_ld_eo(dst, rw, (o + lo) // 128, (o + hi) // 128) - m) * rs)
                ops = _a_ops(*q4)
                yield _or_all([_st_eo(a_ref, t, lo, g * RG, ops[t]) for t in range(7)]) & zmask

    def z2_steps(i, fence):
        for g in range(NG):
            rq = pl.multiple_of(i * H + g * RG, RG)
            fence()
            st = []
            for hh in range(2):
                def row(k):
                    return pl.multiple_of(hh * H + g * RG + zsc[k] * RG, RG)
                m = jnp.mean(_ld_eo(zs, row(0), 0, FH // 128), axis=-1, keepdims=True)
                xc = _ld_eo(zs, row(1), 0, FH // 128) - m
                v = jnp.mean(xc * xc, axis=-1, keepdims=True)
                st.append((row(2), m, jax.lax.rsqrt(v + EPS)))
            yield (_stat_dep(st[0][2]) | _stat_dep(st[1][2])) & zmask
            for (lo, hi) in _chunks(FQ, ZW):
                q4 = []
                for hh in range(2):
                    rw, m, rs = st[hh]
                    for o in (0, FQ):
                        q4.append((_ld_eo(zs, rw, (o + lo) // 128, (o + hi) // 128) - m) * rs)
                ops = _b_ops(*q4)
                yield _or_all([_st_eo(z2ops, t, lo, rq, ops[t]) for t in range(7)]) & zmask

    def spread(nsteps, first, last):
        return [first + (k * (last - first)) // max(nsteps - 1, 1) for k in range(nsteps)]

    def mm1(i, a_ref, inext, src, dst, a_next):
        r = pl.multiple_of(i * TM, TM)
        hist = []

        def fence():
            if len(hist) >= ZK:
                zs[FH // 128 + zsc[0], 0:8, :] = hist[-ZK][0:8, 0:128]

        def half(off, steps, slots, store):
            slot = 0
            for (lo, hi) in _chunks(FQ, TN):
                m = []
                for t in range(7):
                    deps = []
                    for _ in range((hi - lo) // 128):
                        d = None
                        while slots and slots[0] <= slot:
                            slots.pop(0)
                            dn = next(steps)
                            d = dn if d is None else d | dn
                        deps.append(d)
                        slot += 1
                    m.append(_dot(_ld(a_ref, t, 0, D2), _ldg(win_s, t, off + lo, off + hi, deps)))
                    hist.append(m[-1])
                c11, c12, c21, c22 = _c_blocks(m)
                store(0, lo, hi, _gelu(c11))
                store(0, FQ + lo, FQ + hi, _gelu(c12))
                store(1, lo, hi, _gelu(c21))
                store(1, FQ + lo, FQ + hi, _gelu(c22))

        def store_z2(hh, lo, hi, val):
            for c in range(lo // 128, hi // 128):
                zs[c, hh * H:(hh + 1) * H, :] = val[:, c * 128 - lo:(c + 1) * 128 - lo]

        def store_z1(hh, lo, hi, val):
            z1buf[pl.ds(pl.multiple_of(i * H + hh * (H // 2), H // 2), H // 2), lo:hi] = _pk(val[:H // 2], val[H // 2:])

        half(FQ, prologue_steps(inext, src, dst, a_next),
             spread(NG * (2 + len(_chunks(D2, PW))), PA[0], PA[1]), store_z2)
        del hist[:]
        half(0, z2_steps(i, fence), spread(NG * (1 + len(_chunks(FQ, ZW))), ZA[0], ZA[1]), store_z1)

    def build_ws(i, ws_ref):
        G = 32
        for g in range(H // G):
            r1 = pl.ds(pl.multiple_of(i * TM + g * G, G), G)
            r2 = pl.ds(pl.multiple_of(i * TM + H + g * G, G), G)
            for t in range(NT):
                raw = [pltpu.bitcast(wsp_raw[rr, c0:c0 + H], u32)
                       for rr in (r1, r2) for c0 in (t * TM, t * TM + H)]
                ev = _a_ops(*[_unpk(x, 0) for x in raw])
                od = _a_ops(*[_unpk(x, 1) for x in raw])
                for u in range(7):
                    if u == 2:
                        val = raw[0]
                    elif u == 3:
                        val = raw[3]
                    else:
                        val = _pk(ev[u], od[u])
                    ws_ref[u, g * G // 2:(g + 1) * G // 2, t * H:(t + 1) * H] = val

    def mm23(i, ws_ref, src, store):
        r = pl.multiple_of(i * TM, TM)
        for (lo, hi) in _chunks(FQ, TN):
            wdt = hi - lo
            m = [_dot(_ld(ws_ref, t, 0, S // 2), _ld(z2ops, t, lo, hi)) for t in range(7)]
            c11, c12, c21, c22 = _c_blocks(m)
            b1 = jnp.concatenate([bcol[pl.ds(r, H), :]] * (wdt // 128), axis=1)
            b2 = jnp.concatenate([bcol[pl.ds(r + H, H), :]] * (wdt // 128), axis=1)
            def z1(hh, c0):
                w = z1buf[pl.ds(pl.multiple_of(i * H + hh * (H // 2), H // 2), H // 2), c0:c0 + wdt]
                return jnp.concatenate([_unpk(w, 0), _unpk(w, 1)], axis=0)
            p11 = z1(0, lo) * (c11 + b1)
            p12 = z1(0, FQ + lo) * (c12 + b1)
            p21 = z1(1, lo) * (c21 + b2)
            p22 = z1(1, FQ + lo) * (c22 + b2)
            ops = _a_ops(p11, p12, p21, p22)
            for t in range(7):
                _st(pa, t, lo, 0, ops[t].astype(bf16))
        build_ws(jnp.minimum(i + 1, NT - 1), ws_ref)
        for (lo, hi) in _chunks(D2, TN):
            m = [_dot(_ld(pa, t, 0, FQ), wout_b(t, lo, hi)) for t in range(7)]
            c11, c12, c21, c22 = _c_blocks(m)
            def res(hh, c0):
                return jnp.concatenate([src[c, pl.ds(r + hh * H, H), :]
                                        for c in range(c0 // 128, (c0 + hi - lo) // 128)], axis=1)
            store(0, lo, hi, res(0, lo) + c11)
            store(0, D2 + lo, D2 + hi, res(0, D2 + lo) + c12)
            store(1, lo, hi, res(1, lo) + c21)
            store(1, D2 + lo, D2 + hi, res(1, D2 + lo) + c22)

    def out_copy(i, slot):
        r = pl.multiple_of(i * TM, TM)
        return pltpu.make_async_copy(obuf.at[slot], out_hbm.at[pl.ds(r, TM), :], sem_out.at[slot])

    for layer in range(2):
        src = qbuf if layer == 0 else xb
        dst = xa

        for _ in prologue_steps(0, src, dst, a0):
            pass

        def p1_body(ii, carry, src=src, dst=dst, layer=layer):
            i = 2 * ii
            if layer == 0:
                @pl.when(ii == 1)
                def _():
                    q_copy1.wait()
                    wout_copy.start()
                    wsp_copy.start()
            mm1(i, a0, i + 1, src, dst, a1)
            mm1(i + 1, a1, jnp.minimum(i + 2, NT - 1), src, dst, a0)
            return carry

        with jax.named_scope(f'p1_{layer}'):
            jax.lax.fori_loop(0, NT // 2, p1_body, 0)

        if layer == 0:
            wout_copy.wait()
            wsp_copy.wait()
            RB = 64

            def wout_presum(g, carry):
                r = pl.multiple_of(g * RB, RB)
                b11 = wout_raw[pl.ds(r, RB), 0:D2].astype(f32)
                b12 = wout_raw[pl.ds(r, RB), D2:D].astype(f32)
                b21 = wout_raw[pl.ds(FQ + r, RB), 0:D2].astype(f32)
                b22 = wout_raw[pl.ds(FQ + r, RB), D2:D].astype(f32)
                ops = _b_ops(b11, b12, b21, b22)
                for t in range(7):
                    _st(wout_s, t, 0, r, ops[t].astype(bf16))
                return carry
            with jax.named_scope('wout_presum'):
                jax.lax.fori_loop(0, FQ // RB, wout_presum, 0)

        build_ws(0, ws0)

        if layer == 0:
            def p2_body(i, carry):
                r = pl.multiple_of(i * TM, TM)

                def store(hh, lo, hi, val):
                    for c in range(lo // 128, hi // 128):
                        xb[c, pl.ds(r + hh * H, H), :] = val[:, c * 128 - lo:(c + 1) * 128 - lo]
                mm23(i, ws0, xa, store)
                return carry
            with jax.named_scope(f'p2_{layer}'):
                jax.lax.fori_loop(0, NT, p2_body, 0)
        else:
            def p2_body(i, carry):
                slot = i % 2

                def store(hh, lo, hi, val):
                    obuf[slot, hh * H:(hh + 1) * H, lo:hi] = val.astype(bf16)

                @pl.when(i >= 2)
                def _():
                    out_copy(i - 2, slot).wait()
                mm23(i, ws0, xa, store)
                out_copy(i, slot).start()
                return carry
            with jax.named_scope(f'p2_{layer}'):
                jax.lax.fori_loop(0, NT, p2_body, 0)
            out_copy(NT - 2, 0).wait()
            out_copy(NT - 1, 1).wait()


@jax.jit
def pallas_interleave_layers__ssm_conv_h3__mixer_gmlp__prompt_kernel(
    A_q: jax.Array,
    A_k: jax.Array,
    A_v: jax.Array,
    A_shift_k: jax.Array,
    A_ssm_k: jax.Array,
    A_ssm_D: jax.Array,
    B_x: jax.Array,
    B_w_in: jax.Array,
    B_w_sp: jax.Array,
    B_b_sp: jax.Array,
    B_w_out: jax.Array,
):
    fwd_np, inv_np = _dft_mats()
    fwd = jnp.asarray(fwd_np)
    inv = jnp.asarray(inv_np)
    e32 = np.eye(32, dtype=np.float32)[np.arange(32).reshape(2, 8, 2).transpose(0, 2, 1).reshape(-1)]
    z32 = np.zeros((32, 32), np.float32)
    sel = jnp.asarray(_pack_rows(np.block([
        [e32, z32, z32, e32],
        [z32, e32, z32, -e32],
        [-e32, z32, e32, z32],
        [e32, e32, z32, z32],
        [z32, z32, e32, e32],
    ])))
    zero = jnp.asarray(np.zeros((8,), np.int32))

    any_spec = pl.BlockSpec(memory_space=pl.ANY)
    smem_spec = pl.BlockSpec(memory_space=pltpu.SMEM)

    scratch = [
        pltpu.VMEM((NB, S, 128), bf16),
        pltpu.VMEM((NB, S, 128), bf16),
        pltpu.VMEM((NB, 128, S), bf16),
        pltpu.VMEM((S, D), bf16),
        pltpu.VMEM((D, F), bf16),
        pltpu.VMEM((7, D2 // 2, FH), u32),
        pltpu.VMEM((S, S), bf16),
        pltpu.VMEM((FH, D), bf16),
        pltpu.VMEM((7, FQ // 2, D2), u32),
        pltpu.VMEM((NB, S, 128), f32),
        pltpu.VMEM((NB, S, 128), f32),
        pltpu.VMEM((NB, S, 128), f32),
        pltpu.VMEM((S // 2, FH), u32),
        pltpu.VMEM((7, S // 4, FQ), u32),
        pltpu.VMEM((FH // 128 + 1, TM, 128), f32),
        pltpu.VMEM((7, H // 2, D2), u32),
        pltpu.VMEM((7, H // 2, D2), u32),
        pltpu.VMEM((7, H // 2, S // 2), u32),
        pltpu.VMEM((7, H // 2, FQ), u32),
        pltpu.VMEM((S, 128), f32),
        pltpu.VMEM((2, TM, D), bf16),
        pltpu.VMEM((S + 8, 128), f32),
        pltpu.VMEM((6, NC, CP, 128), f32),
        pltpu.VMEM((6, NC, CP, 128), f32),
        pltpu.VMEM((NC, C, 128), u32),
        pltpu.VMEM((NC, C, 128), u32),
        pltpu.VMEM((NB, 8, 128), f32),
        pltpu.VMEM((KS, D), bf16),
        pltpu.VMEM((NB, 128), bf16),
        pltpu.VMEM((S // 128, 128), bf16),
        pltpu.VMEM((4, C, C), u32),
        pltpu.VMEM((4, C // 2, 2 * C), u32),
        pltpu.VMEM((80, 128), u32),
        pltpu.SemaphoreType.DMA((NB,)),
        pltpu.SemaphoreType.DMA((NB,)),
        pltpu.SemaphoreType.DMA((4,)),
        pltpu.SemaphoreType.DMA((2,)),
        pltpu.SemaphoreType.DMA((4,)),
        pltpu.SemaphoreType.DMA((3,)),
    ]

    out = pl.pallas_call(
        _kernel,
        in_specs=[smem_spec] + [any_spec] * 13,
        out_specs=any_spec,
        out_shape=jax.ShapeDtypeStruct((S, D), bf16),
        scratch_shapes=scratch,
        compiler_params=pltpu.CompilerParams(vmem_limit_bytes=127 * 1024 * 1024),
    )(
        zero,
        A_q.reshape(S, D), A_k.reshape(S, D), A_v.reshape(S, D),
        A_shift_k.T, A_ssm_k.reshape(NB, 128, S), A_ssm_D.reshape(NB, 128),
        B_w_in, B_w_sp, B_b_sp.reshape(S // 128, 128), B_w_out,
        fwd, inv, sel,
    )
    return out.reshape(1, S, D)
```

```python
import numpy as np
import jax
import jax.numpy as jnp
import jax.experimental.pallas as pl
import jax.experimental.pallas.tpu as pltpu

f32 = jnp.float32
bf16 = jnp.bfloat16
u32 = jnp.uint32

S = 2048
D = 1024
F = 3584
FH = F // 2
FQ = FH // 2
D2 = D // 2
C = 128
NC = S // C
NB = D // 128
TM = 256
H = TM // 2
NT = S // TM
EPS = 1e-5
KS = 4
TN = 256
WR = D2 // NB
PG = 4
CP = C + 8
LEAD = 3
STR = 0.85
ZK = 3
PW = 256
ZW = 256
PA = (5, 48)
ZA = (7, 48)
PC = 40
SL1 = 2
P0 = 8
RQ = 63
RN = 4
QA = (3, 46)
SL3 = 7
BG = 32
BA = (2, 26)
SL2 = 8
PT = tuple(range(7))
ZT = tuple(range(7))
WT = tuple(range(7))
WRB = 16
WC = 256
WA = (3, 44)
NQ0 = 2
K1 = 2
SUMS = (0, 2, 3, 5, 6)


def _pack_rows(m):
    b = m.astype(bf16).view(np.uint16).astype(np.uint32)
    return b[0::2] | (b[1::2] << 16)


def _dft_mats():
    f = np.arange(C, dtype=np.float64)
    b = np.arange(C, dtype=np.float64)
    perm_f = np.concatenate([np.concatenate([np.arange(8 * p, 8 * p + 8), C + np.arange(8 * p, 8 * p + 8)])
                             for p in range(C // 8)])
    perm_i = np.stack([np.arange(C), C + np.arange(C)], axis=1).reshape(-1)
    fwds, invs = [], []
    for a in range(2):
        ang = 2.0 * np.pi * (f[:, None] + 0.5) * (b[None, :] + C * a) / (2 * C)
        fwd = np.concatenate([np.cos(ang), -np.sin(ang)], axis=0)
        inv = (fwd.T / C)[:, perm_i]
        fwds.append(_pack_rows(fwd[perm_f].astype(np.float32)))
        invs.append(_pack_rows(inv.astype(np.float32)))
    return np.stack(fwds), np.stack(invs)


def _ln(x):
    m = jnp.mean(x, axis=-1, keepdims=True)
    xc = x - m
    v = jnp.mean(xc * xc, axis=-1, keepdims=True)
    return xc * jax.lax.rsqrt(v + EPS)


def _gelu(x):
    c0 = 0.7978845608028654
    inner = x * (c0 + (c0 * 0.044715) * (x * x))
    return x + x * jnp.tanh(inner)


def _dot(a, b):
    return jnp.dot(a, b, preferred_element_type=f32)


def _a_ops(a11, a12, a21, a22):
    return (a11 + a22, a21 + a22, a11, a22, a11 + a12, a21 - a11, a12 - a22)


def _b_ops(b11, b12, b21, b22):
    return (b11 + b22, b11, b12 - b22, b21 - b11, b22, b11 + b12, b21 + b22)


def _c_blocks(m):
    c11 = m[0] + m[3] - m[4] + m[6]
    c12 = m[2] + m[4]
    c21 = m[1] + m[3]
    c22 = m[0] - m[1] + m[2] + m[5]
    return c11, c12, c21, c22


def _chunks(n, w):
    out = []
    o = 0
    while o < n:
        e = min(n, o + w)
        out.append((o, e))
        o = e
    return out


def _gate(x, dep):
    if dep is None:
        return x
    if x.shape[0] == 8:
        return x | dep
    return jnp.concatenate([x[0:8] | dep, x[8:]], axis=0)


def _ld(ref, t, lo, hi):
    return pltpu.bitcast(ref[t, :, lo:hi], bf16)


def _st(ref, t, col0, row0, val):
    n, w = val.shape
    if isinstance(row0, int):
        rows = slice(row0 // 2, (row0 + n) // 2)
    else:
        rows = pl.ds(pl.multiple_of(row0 // 2, 8), n // 2)
    if isinstance(col0, int):
        cols = slice(col0, col0 + w)
    else:
        cols = pl.ds(pl.multiple_of(col0, 128), w)
    pk = pltpu.bitcast(val, jnp.uint32)
    ref[t, rows, cols] = pk
    return pk


def _pk(e, o):
    return pltpu.bitcast(pltpu.pack_elementwise([e, o], packed_dtype=bf16), u32)


def _unpk(u, idx):
    return pltpu.unpack_elementwise(u, index=idx, packed_dtype=bf16, unpacked_dtype=f32)


def _ld_eo(ref, r, c0, c1):
    return jnp.concatenate(
        [jnp.concatenate([ref[c, pl.ds(r, 8, stride=2), :], ref[c, pl.ds(r + 1, 8, stride=2), :]], axis=0)
         for c in range(c0, c1)], axis=1)


def _st_eo(ref, t, col0, row0, val):
    pk = _pk(val[0:8], val[8:16])
    rows = slice(row0 // 2, row0 // 2 + 8) if isinstance(row0, int) else pl.ds(pl.multiple_of(row0 // 2, 8), 8)
    ref[t, rows, col0:col0 + val.shape[1]] = pk
    return pk


def _or_all(vals):
    parts = []
    for v in vals:
        for r in range(0, v.shape[0], 8):
            for c in range(0, v.shape[1], 128):
                parts.append(v[r:r + 8, c:c + 128])
    while len(parts) > 1:
        parts = [parts[i] | parts[i + 1] if i + 1 < len(parts) else parts[i] for i in range(0, len(parts), 2)]
    return parts[0]


def _gate_cols(w, deps):
    nk, nn = w.shape[0] // 64, w.shape[1] // 128
    tiles = [(k, j) for j in range(nn) for k in range(nk)]
    at = {tiles[(q * len(tiles)) // len(deps)]: d for q, d in enumerate(deps) if d is not None}
    parts = []
    for k in range(nk):
        if any((k, j) in at for j in range(nn)):
            top = [w[64 * k:64 * k + 8, j * 128:(j + 1) * 128] for j in range(nn)]
            top = [x | at[k, j] if (k, j) in at else x for j, x in enumerate(top)]
            parts += [top[0] if nn == 1 else jnp.concatenate(top, axis=1), w[64 * k + 8:64 * k + 64]]
        else:
            parts.append(w[64 * k:64 * k + 64])
    return pltpu.bitcast(jnp.concatenate(parts, axis=0) if at else w, bf16)


def _stat_dep(x):
    b = pltpu.bitcast(jnp.broadcast_to(x, (16, 128)), u32)
    return b[0:8] | b[8:16]


def _kernel(zero_ref, q_hbm, k_hbm, v_hbm, sk_hbm, h_hbm, dd_hbm, win_hbm, wsp_hbm, bsp_hbm, wout_hbm,
            fwd_hbm, inv_hbm,
            out_hbm,
            kbuf, vbuf, hbuf, qbuf, win_raw, win_s, wsp_raw, wout_raw, wout_s,
            ybuf, xa, xb, z1buf, z2ops, zs, a0, a1, ws0, pa, bcol, obuf,
            kf, spA, spB, wscA, wscB, cpar,
            sk_ref, dd_ref, bsp_ref, fwd_ref, inv_ref,
            sem_kvh, sem_win, sem_misc, sem_out, sem_q0, sem_small):

    def kvh_copies(c):
        cols = pl.ds(pl.multiple_of(c * 128, 128), 128)
        return (
            pltpu.make_async_copy(k_hbm.at[:, cols], kbuf.at[c], sem_kvh.at[c]),
            pltpu.make_async_copy(v_hbm.at[:, cols], vbuf.at[c], sem_kvh.at[c]),
            pltpu.make_async_copy(h_hbm.at[c], hbuf.at[c], sem_kvh.at[c]),
        )

    def win_copies(c):
        r1 = pl.ds(pl.multiple_of(c * WR, WR), WR)
        r2 = pl.ds(pl.multiple_of(D2 + c * WR, WR), WR)
        return (
            pltpu.make_async_copy(win_hbm.at[r1, :], win_raw.at[r1, :], sem_win.at[c]),
            pltpu.make_async_copy(win_hbm.at[r2, :], win_raw.at[r2, :], sem_win.at[c]),
        )

    QS = 3 * TM
    q_copy0 = pltpu.make_async_copy(q_hbm.at[0:TM, :], qbuf.at[0:TM, :], sem_misc.at[0])
    q_copy0b = pltpu.make_async_copy(q_hbm.at[TM:QS, :], qbuf.at[TM:QS, :], sem_misc.at[4])
    q_copy1 = pltpu.make_async_copy(q_hbm.at[QS:S, :], qbuf.at[QS:S, :], sem_misc.at[3])
    wout_copy = pltpu.make_async_copy(wout_hbm, wout_raw, sem_misc.at[1])
    wsp_copy = pltpu.make_async_copy(wsp_hbm, wsp_raw, sem_misc.at[2])

    def start_all(cps):
        for cp in cps:
            cp.start()

    def wait_all(cps):
        for cp in cps:
            cp.wait()

    def kvh0_copies(it):
        rows = pl.ds(pl.multiple_of(it * (S // 4), S // 4), S // 4)
        return (
            pltpu.make_async_copy(k_hbm.at[rows, 0:128], kbuf.at[0, rows, :], sem_q0.at[it]),
            pltpu.make_async_copy(v_hbm.at[rows, 0:128], vbuf.at[0, rows, :], sem_q0.at[it]),
            pltpu.make_async_copy(h_hbm.at[0, :, rows], hbuf.at[0, :, rows], sem_q0.at[it]),
        )

    small0 = (
        pltpu.make_async_copy(sk_hbm, sk_ref, sem_small.at[0]),
        pltpu.make_async_copy(dd_hbm, dd_ref, sem_small.at[0]),
    )
    fwd_copy = pltpu.make_async_copy(fwd_hbm, fwd_ref.at[0:2], sem_small.at[1])
    small2 = (
        pltpu.make_async_copy(inv_hbm, inv_ref.at[0:2], sem_small.at[2]),
        pltpu.make_async_copy(bsp_hbm, bsp_ref, sem_small.at[2]),
    )

    start_all(small0)
    fwd_copy.start()
    for it in range(NQ0):
        start_all(kvh0_copies(it))
    wait_all(small0)
    fwd_copy.wait()
    for it in range(NQ0, 4):
        start_all(kvh0_copies(it))
    start_all(small2)

    sign = jnp.uint32(0x80008000)
    fwd_ref[2:4] = fwd_ref[0:2] ^ sign
    skf = sk_ref[...].astype(f32)
    ddf = dd_ref[...].astype(f32)
    for c in range(NB):
        cpar[c, 0:KS, :] = skf[:, c * 128:(c + 1) * 128]
        cpar[c, KS:KS + 1, :] = ddf[c:c + 1, :]

    def win_presum(c, it, dep):
        RG = 32
        g, half, cb = it // 14, (it // 7) % 2, it % 7
        r = pl.multiple_of(c * WR + g * RG, RG)
        r2 = pl.multiple_of(D2 + c * WR + g * RG, RG)
        o = half * FH + cb * 128
        b11 = pltpu.bitcast(win_raw[pl.ds(r, RG), o:o + 128], u32)
        b12 = pltpu.bitcast(win_raw[pl.ds(r, RG), o + FQ:o + FQ + 128], u32)
        b21 = pltpu.bitcast(win_raw[pl.ds(r2, RG), o:o + 128], u32)
        b22 = pltpu.bitcast(win_raw[pl.ds(r2, RG), o + FQ:o + FQ + 128], u32)
        raw = [_gate(x, dep) for x in (b11, b12, b21, b22)]
        ev = _b_ops(*[_unpk(x, 0) for x in raw])
        od = _b_ops(*[_unpk(x, 1) for x in raw])
        col = half * FQ + cb * 128
        rows = pl.ds(pl.multiple_of(c * (WR // 2) + g * (RG // 2), RG // 2), RG // 2)
        for t in range(7):
            win_s[t, rows, col:col + 128] = _pk(ev[t], od[t]) if t in SUMS else raw[t - 1]

    zsc = [zero_ref[g] for g in range(NC // PG)]
    zmask = jnp.full((8, 128), zsc[0], jnp.int32).astype(u32)

    def conv_stage(c, par, do_prod, do_fwd, do_inv, chunks=range(NC), a0=0, pre=(), mid=None):
        sp_cur, sp_nxt = (spA, spB) if par == 0 else (spB, spA)
        ws_cur, ws_prv = (wscA, wscB) if par == 0 else (wscB, wscA)
        cn, cp = c + 1, c - 1

        def crow(a, off=0, n=C):
            if isinstance(a0, int):
                return slice((a0 + a) * n + off, (a0 + a + 1) * n + off)
            return pl.ds(pl.multiple_of(a0 * n, n) + (a * n + off), n)

        fin = []

        def inv(a, dep):
            wv = ws_prv[a0 + a]
            wv = jnp.concatenate([_gate(wv[:C // 2], dep), _gate(wv[C // 2:], dep)], axis=0)
            y = _dot(pltpu.bitcast(inv_ref[a % 4], bf16), pltpu.bitcast(wv, bf16))
            ybuf[cp, crow(a), :] = y
            fin.append(pltpu.bitcast(y[C - 8:C], u32))

        def hf(a, dep):
            hv = hbuf[cn, :, crow(a)]
            if dep is not None:
                hv = pltpu.bitcast(_gate(pltpu.bitcast(hv, u32), dep), bf16)
            hj = jax.lax.dot_general(pltpu.bitcast(fwd_ref[a % 4], bf16), hv,
                                     (((1,), (1,)), ((), ())), preferred_element_type=f32)
            if a == 0:
                dd = cpar[cn, KS:KS + 1, :]
                if not isinstance(a0, int):
                    dd = jnp.where(a0 == 0, dd, 0.0)
            for p in range(C // 8):
                re = hj[16 * p:16 * p + 8]
                im = hj[16 * p + 8:16 * p + 16]
                if a == 0:
                    re = re + dd
                sp_nxt[3, a0 + a, 8 * p:8 * p + 8, :] = re
                sp_nxt[4, a0 + a, 8 * p:8 * p + 8, :] = im - re
                sp_nxt[5, a0 + a, 8 * p:8 * p + 8, :] = im + re
            fin.append(pltpu.bitcast(im, u32))

        def uf(a, dep):
            w = [cpar[cn, t:t + 1, :] for t in range(KS)]
            k0 = pltpu.bitcast(kbuf[cn, crow(a), :], u32)
            kf[crow(a, 8, C // 2), :] = k0
            k1 = kf[crow(a, 7, C // 2), :]
            ke, ko, ke1, ko1 = _unpk(k0, 0), _unpk(k0, 1), _unpk(k1, 0), _unpk(k1, 1)
            ko2 = _unpk(kf[crow(a, 6, C // 2), :], 1)
            vw = pltpu.bitcast(vbuf[cn, crow(a), :], u32)
            kse = w[0] * ke + w[1] * ko1 + w[2] * ke1 + w[3] * ko2
            kso = w[0] * ko + w[1] * ke + w[2] * ko1 + w[3] * ke1
            kv = _gate(_pk(kse * _unpk(vw, 0), kso * _unpk(vw, 1)), dep)
            u = _dot(pltpu.bitcast(fwd_ref[a % 4], bf16), pltpu.bitcast(kv, bf16))
            for p in range(C // 8):
                re = u[16 * p:16 * p + 8]
                im = u[16 * p + 8:16 * p + 16]
                sp_nxt[0, a0 + a, 8 * p:8 * p + 8, :] = im + re
                sp_nxt[1, a0 + a, 8 * p:8 * p + 8, :] = re
                sp_nxt[2, a0 + a, 8 * p:8 * p + 8, :] = im
            fin.append(pltpu.bitcast(im, u32))

        prev = {}

        def pgroup(p, g, dep):
            rows = pl.ds(pl.multiple_of(p * 8 + zsc[g] * 8, 8), 8)
            outs = range(g * PG, (g + 1) * PG)
            acc, hw = {}, {}
            for j in range((g + 1) * PG):
                uu = [sp_cur[k, j, rows, :] for k in range(3)]
                if j == 0 and dep is not None:
                    uu = [pltpu.bitcast(_gate(pltpu.bitcast(x, u32), dep), f32) for x in uu]
                for a in outs:
                    l = a - j
                    if l < 0:
                        continue
                    if l not in hw:
                        hw[l] = [sp_cur[3 + k, l, rows, :] for k in range(3)]
                    for k in range(3):
                        pr = hw[l][k] * uu[k]
                        acc[a, k] = pr if (a, k) not in acc else acc[a, k] + pr
            d = None
            for a in outs:
                re = acc[a, 0] - acc[a, 2]
                im = acc[a, 0] + acc[a, 1]
                if a == 0:
                    wr, wi = re, im
                else:
                    wr, wi = re + prev['re'], im + prev['im']
                prev['re'], prev['im'] = re, im
                pk = pltpu.bitcast(pltpu.pack_elementwise([wr, wi], packed_dtype=bf16), u32)
                ws_cur[a, p * 8:p * 8 + 8, :] = pk
                if a % 2 == 1:
                    d = pk if d is None else d | pk
            return d & zmask

        dots = []
        for a in chunks:
            if do_fwd:
                dots += [(uf, a), (hf, a)]
            if do_inv:
                dots += [(inv, a)]
            for cw in pre:
                dots += [(lambda it, dep, cw=cw: win_presum(cw, it, dep), it)
                         for it in range(a * 28 // NC, (a + 1) * 28 // NC)]
        cost = [PC if fn not in (uf, hf, inv) else 256 for fn, _ in dots]
        pos = (np.cumsum(cost) - cost - LEAD * 256) / sum(cost) * STR
        nd = len(dots)
        if not do_prod:
            for fn, a in dots:
                fn(a, None)
            return
        ng = NC // PG
        wts = [sum(a + 1 for a in range(g * PG, (g + 1) * PG)) for g in range(ng)] * (C // 8)
        cum = np.cumsum(wts) / sum(wts)
        i0 = 0 if mid is None else P0 * ng
        base = 0.0 if i0 == 0 else cum[i0 - 1]
        cum = (cum - base) / (1.0 - base)
        d = 0
        dep = None
        i = 0
        for p in range(C // 8):
            for g in range(ng):
                if i == i0:
                    if mid is not None:
                        mid()
                    while d < nd and pos[d] <= 0:
                        dots[d][0](dots[d][1], None)
                        d += 1
                if i == RQ:
                    assert d == nd
                    dep = dep | (_or_all(fin[-RN:]) & zmask)
                dep = pgroup(p, g, dep)
                while i >= i0 and d < nd and pos[d] <= cum[i]:
                    dots[d][0](dots[d][1], dep)
                    d += 1
                i += 1

    kf[0:8, :] = jnp.zeros((8, 128), u32)

    with jax.named_scope('conv'):
        def first_body(it, carry):
            wait_all(kvh0_copies(it))

            @pl.when(it == K1)
            def _():
                start_all(kvh_copies(1))
            conv_stage(-1, 1, False, True, False, range(4), it * 4)
            return carry
        jax.lax.fori_loop(0, NC // 4, first_body, 0)
        xb[:, 0:TM, :] = jnp.zeros((NB, TM, 128), f32)
        wait_all(small2)
        inv_ref[2:4] = inv_ref[0:2] ^ sign
        for r in range(S // 128):
            row = bsp_ref[r:r + 1, :].astype(f32)
            bcol[r * 128:(r + 1) * 128, :] = 0.5 * jnp.broadcast_to(row, (128, 128)).T

        def mid0():
            wait_all(kvh_copies(1)[:2])
            start_all(kvh_copies(2))
            wait_all(kvh_copies(1)[2:])
        conv_stage(0, 0, True, True, False, mid=mid0)

        def conv_body(ii, carry):
            for e in range(2):
                c = 2 * ii + 1 + e
                if e == 0:
                    @pl.when(c >= 2)
                    def _():
                        wait_all(win_copies(c - 2))
                    wait_all(kvh_copies(c + 1)[:2])
                    start_all(kvh_copies(c + 2))
                    start_all(win_copies(c - 1))
                    cw = jnp.where(c >= 2, c - 2, NB - 1)
                else:
                    wait_all(win_copies(c - 2))
                    wait_all(kvh_copies(c + 1)[:2])

                    @pl.when(c + 2 < NB)
                    def _():
                        start_all(kvh_copies(c + 2))

                    @pl.when(c + 2 == NB)
                    def _():
                        start_all(win_copies(c))
                        q_copy0.start()
                    start_all(win_copies(c - 1))
                    cw = c - 2
                wait_all(kvh_copies(c + 1)[2:])
                conv_stage(c, 1 - e, True, True, True, pre=(cw,))
            return carry
        jax.lax.fori_loop(0, NB // 2 - 1, conv_body, 0)
        wait_all(win_copies(NB - 3))
        start_all(win_copies(NB - 1))
        q_copy0b.start()
        wait_all(win_copies(NB - 2))
        conv_stage(NB - 1, 1, True, False, True, pre=(NB - 3, NB - 2))

    q_copy0.wait()
    wait_all(win_copies(NB - 1))

    conv_stage(NB, 0, False, False, True)
    for it in range(28):
        win_presum(NB - 1, it, None)

    def wout_b(t, lo, hi):
        if t == 1:
            return pltpu.bitcast(wout_raw[0:FQ, lo:hi], u32)
        if t == 4:
            return pltpu.bitcast(wout_raw[FQ:FH, D2 + lo:D2 + hi], u32)
        return wout_s[SUMS.index(t), :, lo:hi]

    RG = 16
    NG = H // RG

    def a_buf(ref):
        return (lambda t: _ld(ref, t, 0, D2)), (lambda t, lo, g, val: _st_eo(ref, t, lo, g * RG, val))

    def prologue_steps(i, src, a_st, groups=range(NG), idst=None):
        for g in groups:
            st = []
            for hh in range(2):
                r = pl.multiple_of(i * TM + hh * H + g * RG, RG)
                rd = r if idst is None else pl.multiple_of(idst * TM + hh * H + g * RG, RG)
                if src is qbuf:
                    xq = pltpu.bitcast(src[pl.ds(r, RG), :], u32)
                    x = jnp.concatenate([_unpk(xq, 0), _unpk(xq, 1)], axis=0)
                else:
                    x = _ld_eo(src, r, 0, NB)
                x1 = x + _ln(x) * _ld_eo(ybuf, r, 0, NB)
                for c in range(NB):
                    xa[c, pl.ds(rd, 8, stride=2), :] = x1[0:8, c * 128:(c + 1) * 128]
                    xa[c, pl.ds(rd + 1, 8, stride=2), :] = x1[8:16, c * 128:(c + 1) * 128]
                m = jnp.mean(x1, axis=-1, keepdims=True)
                xc = x1 - m
                rs = jax.lax.rsqrt(jnp.mean(xc * xc, axis=-1, keepdims=True) + EPS)
                st.append((pl.multiple_of((i if idst is None else idst) * TM + hh * H + g * RG + zsc[1] * RG, RG), m, rs))
                yield _stat_dep(rs) & zmask
            for (lo, hi) in _chunks(D2, PW):
                q4 = []
                for hh in range(2):
                    rw, m, rs = st[hh]
                    for o in (0, D2):
                        q4.append((_ld_eo(xa, rw, (o + lo) // 128, (o + hi) // 128) - m) * rs)
                ops = _a_ops(*q4)
                yield _or_all([a_st(t, lo, g, ops[t]) for t in range(7)]) & zmask

    def prologue0(a_st):
        def row(j, k):
            return pl.multiple_of(j * RG + zsc[k] * RG, RG)

        def ldq(j, k):
            xq = pltpu.bitcast(qbuf[pl.ds(row(j, k), RG), :], u32)
            return jnp.concatenate([_unpk(xq, 0), _unpk(xq, 1)], axis=0)

        def rstd(xc):
            return jax.lax.rsqrt(jnp.mean(xc * xc, axis=-1, keepdims=True) + EPS)
        js = range(2 * NG)
        m1 = [jnp.mean(ldq(j, 0), axis=-1, keepdims=True) for j in js]
        r1 = [rstd(ldq(j, 1) - m1[j]) for j in js]
        m2 = []
        for j in js:
            x = ldq(j, 2)
            x1 = x + (x - m1[j]) * r1[j] * _ld_eo(ybuf, j * RG, 0, NB)
            for c in range(NB):
                xa[c, pl.ds(j * RG, 8, stride=2), :] = x1[0:8, c * 128:(c + 1) * 128]
                xa[c, pl.ds(j * RG + 1, 8, stride=2), :] = x1[8:16, c * 128:(c + 1) * 128]
            m2.append(jnp.mean(x1, axis=-1, keepdims=True))
        r2 = [rstd(_ld_eo(xa, row(j, 0), 0, NB) - m2[j]) for j in js]
        for g in range(NG):
            for (lo, hi) in _chunks(D2, PW):
                q4 = [(_ld_eo(xa, row(j, 1), (o + lo) // 128, (o + hi) // 128) - m2[j]) * r2[j]
                      for j in (g, NG + g) for o in (0, D2)]
                ops = _a_ops(*q4)
                for t in range(7):
                    a_st(t, lo, g, ops[t])

    PS = 2 + len(_chunks(D2, PW))

    def z2_steps(i, fence):
        for g in range(NG):
            rq = pl.multiple_of(i * H + g * RG, RG)
            fence()
            st = []
            for hh in range(2):
                def row(k):
                    return pl.multiple_of(hh * H + g * RG + zsc[k] * RG, RG)
                m = jnp.mean(_ld_eo(zs, row(0), 0, FH // 128), axis=-1, keepdims=True)
                xc = _ld_eo(zs, row(1), 0, FH // 128) - m
                v = jnp.mean(xc * xc, axis=-1, keepdims=True)
                st.append((row(2), m, 0.5 * jax.lax.rsqrt(v + 4.0 * EPS)))
            yield (_stat_dep(st[0][2]) | _stat_dep(st[1][2])) & zmask
            for (lo, hi) in _chunks(FQ, ZW):
                q4 = []
                for hh in range(2):
                    rw, m, rs = st[hh]
                    for o in (0, FQ):
                        q4.append((_ld_eo(zs, rw, (o + lo) // 128, (o + hi) // 128) - m) * rs)
                ops = _b_ops(*q4)
                yield _or_all([_st_eo(z2ops, t, lo, rq, ops[t]) for t in range(7)]) & zmask

    def spread(nsteps, first, last, sl, ts, n=FQ):
        prod = [t for (lo, hi) in _chunks(n, TN) for t in range(7) for _ in range((hi - lo) // 128 * sl)]
        ok = [q for q, t in enumerate(prod) if first * sl <= q < (last + 1) * sl and t in ts]
        return [ok[(k * (len(ok) - 1)) // max(nsteps - 1, 1)] for k in range(nsteps)]

    def anchors(steps, slots):
        state = [0]

        def take(n):
            deps = []
            for _ in range(n):
                d = None
                while slots and slots[0] <= state[0]:
                    slots.pop(0)
                    dn = next(steps)
                    d = dn if d is None else d | dn
                deps.append(d)
                state[0] += 1
            return deps
        return take

    def wout_steps():
        for g in range(FQ // WRB):
            for (lo, hi) in _chunks(D2, WC):
                raw = [pltpu.bitcast(wout_raw[r0 + g * WRB:r0 + (g + 1) * WRB, c0 + lo:c0 + hi], u32)
                       for r0 in (0, FQ) for c0 in (0, D2)]
                ev = _b_ops(*[_unpk(x, 0) for x in raw])
                od = _b_ops(*[_unpk(x, 1) for x in raw])
                pks = [_pk(ev[t], od[t]) for t in SUMS]
                for k in range(5):
                    wout_s[k, g * WRB // 2:(g + 1) * WRB // 2, lo:hi] = pks[k]
                yield _or_all(pks) & zmask

    def mm1(i, a_ld, psteps, nps):
        hist = []

        def fence():
            if len(hist) >= ZK:
                zs[FH // 128 + zsc[0], 0:8, :] = hist[-ZK][0:8, 0:128]

        def half(off, steps, slots, store):
            take = anchors(steps, slots)
            for (lo, hi) in _chunks(FQ, TN):
                m = []
                for t in range(7):
                    deps = take((hi - lo) // 128 * SL1)
                    m.append(_dot(a_ld(t), _gate_cols(win_s[t, :, off + lo:off + hi], deps)))
                    hist.append(m[-1])
                c11, c12, c21, c22 = _c_blocks(m)
                store(0, lo, hi, _gelu(c11))
                store(0, FQ + lo, FQ + hi, _gelu(c12))
                store(1, lo, hi, _gelu(c21))
                store(1, FQ + lo, FQ + hi, _gelu(c22))

        def store_z2(hh, lo, hi, val):
            for c in range(lo // 128, hi // 128):
                zs[c, hh * H:(hh + 1) * H, :] = val[:, c * 128 - lo:(c + 1) * 128 - lo]

        def store_z1(hh, lo, hi, val):
            z1buf[pl.ds(pl.multiple_of(i * H + hh * (H // 2), H // 2), H // 2), lo:hi] = _pk(val[:H // 2], val[H // 2:])

        half(FQ, psteps, spread(nps, PA[0], PA[1], SL1, PT), store_z2)
        del hist[:]
        half(0, z2_steps(i, fence), spread(NG * (1 + len(_chunks(FQ, ZW))), ZA[0], ZA[1], SL1, ZT), store_z1)

    def ws_steps(i, ws_ref):
        G = BG
        for g in range(H // G):
            r1 = pl.ds(pl.multiple_of(i * TM + g * G, G), G)
            r2 = pl.ds(pl.multiple_of(i * TM + H + g * G, G), G)
            for t in range(NT):
                raw = [pltpu.bitcast(wsp_raw[rr, c0:c0 + H], u32)
                       for rr in (r1, r2) for c0 in (t * TM, t * TM + H)]
                ev = _a_ops(*[_unpk(x, 0) for x in raw])
                od = _a_ops(*[_unpk(x, 1) for x in raw])
                vals = [raw[0] if u == 2 else raw[3] if u == 3 else _pk(ev[u], od[u]) for u in range(7)]
                for u in range(7):
                    ws_ref[u + zsc[0], g * G // 2:(g + 1) * G // 2, t * H:(t + 1) * H] = vals[u]
                yield _or_all([vals[u] for u in (0, 1, 4, 5, 6)]) & zmask

    def mm23(i, inext, ws_ref, src, store, take, done=None):
        r = pl.multiple_of(i * TM, TM)
        for (lo, hi) in _chunks(FQ, TN):
            wdt = hi - lo
            m = [_dot(_ld(ws_ref, t, 0, S // 2), _gate_cols(z2ops[t, :, lo:hi], take(wdt // 128 * SL2)))
                 for t in range(7)]
            c11, c12, c21, c22 = _c_blocks(m)
            b1 = jnp.concatenate([bcol[pl.ds(r, H), :]] * (wdt // 128), axis=1)
            b2 = jnp.concatenate([bcol[pl.ds(r + H, H), :]] * (wdt // 128), axis=1)
            def z1(hh, c0):
                w = z1buf[pl.ds(pl.multiple_of(i * H + hh * (H // 2), H // 2), H // 2), c0:c0 + wdt]
                return jnp.concatenate([_unpk(w, 0), _unpk(w, 1)], axis=0)
            p11 = z1(0, lo) * (c11 + b1)
            p12 = z1(0, FQ + lo) * (c12 + b1)
            p21 = z1(1, lo) * (c21 + b2)
            p22 = z1(1, FQ + lo) * (c22 + b2)
            ops = _a_ops(p11, p12, p21, p22)
            for t in range(7):
                _st(pa, t, lo, 0, ops[t].astype(bf16))
        take3 = anchors(ws_steps(inext, ws_ref), spread(H // BG * NT, BA[0], BA[1], SL3, WT, D2))
        for (lo, hi) in _chunks(D2, TN):
            m = [_dot(_ld(pa, t, 0, FQ), _gate_cols(wout_b(t, lo, hi), take3((hi - lo) // 128 * SL3)))
                 for t in range(7)]
            c11, c12, c21, c22 = _c_blocks(m)
            def res(hh, c0):
                return jnp.concatenate([src[c, pl.ds(r + hh * H, H), :]
                                        for c in range(c0 // 128, (c0 + hi - lo) // 128)], axis=1)
            store(0, lo, hi, res(0, lo) + c11)
            store(0, D2 + lo, D2 + hi, res(0, D2 + lo) + c12)
            store(1, lo, hi, res(1, lo) + c21)
            store(1, D2 + lo, D2 + hi, res(1, D2 + lo) + c22)
            if done is not None:
                done(lo)

    def out_copy(i, slot, los=range(0, D2, TN)):
        rows = pl.ds(pl.multiple_of(i * TM, TM), TM)
        return [pltpu.make_async_copy(obuf.at[slot, :, c0:c0 + TN], out_hbm.at[rows, c0:c0 + TN], sem_out.at[slot])
                for lo in los for c0 in (lo, D2 + lo)]

    def merge(steps_a, slots_a, steps_b, slots_b):
        order = sorted([(q, 0) for q in slots_a] + [(q, 1) for q in slots_b])

        def gen():
            for _, w in order:
                yield next(steps_b if w else steps_a)
        return anchors(gen(), [q for q, _ in order])

    (ld0, st0), (ld1, st1) = a_buf(a0), a_buf(a1)
    prologue0(st0)
    q_copy1.start()
    q_copy0b.wait()

    for layer in range(2):
        def p1_body(ii, carry, layer=layer):
            i = 2 * ii
            if layer == 0:
                @pl.when(ii == 1)
                def _():
                    q_copy1.wait()
                    wout_copy.start()
                    wsp_copy.start()
            src = qbuf if layer == 0 else xb
            mm1(i, ld0, prologue_steps(i + 1, src, st1), NG * PS)
            mm1(i + 1, ld1, prologue_steps(jnp.minimum(i + 2, NT - 1), src, st0), NG * PS)
            return carry

        with jax.named_scope(f'p1_{layer}'):
            jax.lax.fori_loop(0, NT // 2, p1_body, 0)

        if layer == 0:
            wout_copy.wait()
            wsp_copy.wait()
            for _ in ws_steps(0, ws0):
                pass

        if layer == 0:
            def p2_body(i, carry):
                r = pl.multiple_of(i * TM, TM)

                def store(hh, lo, hi, val):
                    for c in range(lo // 128, hi // 128):
                        xb[c, pl.ds(r + hh * H, H), :] = val[:, c * 128 - lo:(c + 1) * 128 - lo]
                g0 = 2 * jnp.clip(i - 1, 0, NG // 2 - 1)
                take = merge(wout_steps(), spread(FQ // WRB * (D2 // WC), WA[0], WA[1], SL2, WT),
                             prologue_steps(0, xb, st0, (g0, g0 + 1), jnp.where(i == 0, NT, 0)),
                             spread(2 * PS, QA[0], QA[1], SL2, WT))
                mm23(i, (i + 1) % NT, ws0, xa, store, take)
                return carry
            with jax.named_scope(f'p2_{layer}'):
                jax.lax.fori_loop(0, NT, p2_body, 0)
        else:
            def p2_body(i, carry):
                slot = i % 2

                def store(hh, lo, hi, val):
                    obuf[slot, hh * H:(hh + 1) * H, lo:hi] = val.astype(bf16)

                @pl.when(i >= 2)
                def _():
                    wait_all(out_copy(i - 2, slot))
                mm23(i, (i + 1) % NT, ws0, xa, store, anchors(None, []),
                     lambda lo: start_all(out_copy(i, slot, (lo,))))
                return carry
            with jax.named_scope(f'p2_{layer}'):
                jax.lax.fori_loop(0, NT, p2_body, 0)
            wait_all(out_copy(NT - 2, 0))
            wait_all(out_copy(NT - 1, 1))


@jax.jit
def pallas_interleave_layers__ssm_conv_h3__mixer_gmlp__prompt_kernel(
    A_q: jax.Array,
    A_k: jax.Array,
    A_v: jax.Array,
    A_shift_k: jax.Array,
    A_ssm_k: jax.Array,
    A_ssm_D: jax.Array,
    B_x: jax.Array,
    B_w_in: jax.Array,
    B_w_sp: jax.Array,
    B_b_sp: jax.Array,
    B_w_out: jax.Array,
):
    fwd_np, inv_np = _dft_mats()
    fwd = jnp.asarray(fwd_np)
    inv = jnp.asarray(inv_np)
    zero = jnp.asarray(np.zeros((8,), np.int32))

    any_spec = pl.BlockSpec(memory_space=pl.ANY)
    smem_spec = pl.BlockSpec(memory_space=pltpu.SMEM)

    scratch = [
        pltpu.VMEM((NB, S, 128), bf16),
        pltpu.VMEM((NB, S, 128), bf16),
        pltpu.VMEM((NB, 128, S), bf16),
        pltpu.VMEM((S, D), bf16),
        pltpu.VMEM((D, F), bf16),
        pltpu.VMEM((7, D2 // 2, FH), u32),
        pltpu.VMEM((S, S), bf16),
        pltpu.VMEM((FH, D), bf16),
        pltpu.VMEM((5, FQ // 2, D2), u32),
        pltpu.VMEM((NB, S, 128), f32),
        pltpu.VMEM((NB, S + TM, 128), f32),
        pltpu.VMEM((NB, S, 128), f32),
        pltpu.VMEM((S // 2, FH), u32),
        pltpu.VMEM((7, S // 4, FQ), u32),
        pltpu.VMEM((FH // 128 + 1, TM, 128), f32),
        pltpu.VMEM((7, H // 2, D2), u32),
        pltpu.VMEM((7, H // 2, D2), u32),
        pltpu.VMEM((7, H // 2, S // 2), u32),
        pltpu.VMEM((7, H // 2, FQ), u32),
        pltpu.VMEM((S, 128), f32),
        pltpu.VMEM((2, TM, D), bf16),
        pltpu.VMEM((S // 2 + 8, 128), u32),
        pltpu.VMEM((6, NC + 1, CP, 128), f32),
        pltpu.VMEM((6, NC + 1, CP, 128), f32),
        pltpu.VMEM((NC, C, 128), u32),
        pltpu.VMEM((NC, C, 128), u32),
        pltpu.VMEM((NB, 8, 128), f32),
        pltpu.VMEM((KS, D), bf16),
        pltpu.VMEM((NB, 128), bf16),
        pltpu.VMEM((S // 128, 128), bf16),
        pltpu.VMEM((4, C, C), u32),
        pltpu.VMEM((4, C // 2, 2 * C), u32),
        pltpu.SemaphoreType.DMA((NB,)),
        pltpu.SemaphoreType.DMA((NB,)),
        pltpu.SemaphoreType.DMA((5,)),
        pltpu.SemaphoreType.DMA((2,)),
        pltpu.SemaphoreType.DMA((4,)),
        pltpu.SemaphoreType.DMA((3,)),
    ]

    out = pl.pallas_call(
        _kernel,
        in_specs=[smem_spec] + [any_spec] * 12,
        out_specs=any_spec,
        out_shape=jax.ShapeDtypeStruct((S, D), bf16),
        scratch_shapes=scratch,
        compiler_params=pltpu.CompilerParams(vmem_limit_bytes=127 * 1024 * 1024, disable_bounds_checks=True),
    )(
        zero,
        A_q.reshape(S, D), A_k.reshape(S, D), A_v.reshape(S, D),
        A_shift_k.T, A_ssm_k.reshape(NB, 128, S), A_ssm_D.reshape(NB, 128),
        B_w_in, B_w_sp, B_b_sp.reshape(S // 128, 128), B_w_out,
        fwd, inv,
    )
    return out.reshape(1, S, D)
```

```python
import numpy as np
import jax
import jax.numpy as jnp
import jax.experimental.pallas as pl
import jax.experimental.pallas.tpu as pltpu

f32 = jnp.float32
bf16 = jnp.bfloat16
u32 = jnp.uint32

S = 2048
D = 1024
F = 3584
FH = F // 2
FQ = FH // 2
D2 = D // 2
C = 128
NC = S // C
NB = D // 128
TM = 256
H = TM // 2
NT = S // TM
EPS = 1e-5
KS = 4
TN = 256
WR = D2 // NB
PG = 4
CP = C + 8
LEAD, STR, PC = 3, 0.85, 40
RQ, RN, OS, P0 = 63, 4, 0.85, 8
NQ0, K1 = 2, 2
PW = ZW = WC = 256
WRB, BG, ZK = 16, 32, 3
SL1, SL2, SL3 = 2, 8, 7
PA, ZA, QA, WA, BA = (5, 48), (7, 48), (3, 46), (3, 44), (2, 26)
SUMS = (0, 2, 3, 5, 6)


def _pack_rows(m):
    b = m.astype(bf16).view(np.uint16).astype(np.uint32)
    return b[0::2] | (b[1::2] << 16)


def _dft_mats():
    f = np.arange(C, dtype=np.float64)
    b = np.arange(C, dtype=np.float64)
    perm_f = np.concatenate([np.concatenate([np.arange(8 * p, 8 * p + 8), C + np.arange(8 * p, 8 * p + 8)])
                             for p in range(C // 8)])
    perm_i = np.stack([np.arange(C), C + np.arange(C)], axis=1).reshape(-1)
    fwds, invs = [], []
    for a in range(2):
        ang = 2.0 * np.pi * (f[:, None] + 0.5) * (b[None, :] + C * a) / (2 * C)
        fwd = np.concatenate([np.cos(ang), -np.sin(ang)], axis=0)
        inv = (fwd.T / C)[:, perm_i]
        fwds.append(_pack_rows(fwd[perm_f].astype(np.float32)))
        invs.append(_pack_rows(inv.astype(np.float32)))
    return np.stack(fwds), np.stack(invs)


def _ln(x):
    m = jnp.mean(x, axis=-1, keepdims=True)
    xc = x - m
    v = jnp.mean(xc * xc, axis=-1, keepdims=True)
    return xc * jax.lax.rsqrt(v + EPS)


def _gelu(x):
    c0 = 0.7978845608028654
    inner = x * (c0 + (c0 * 0.044715) * (x * x))
    return x + x * jnp.tanh(inner)


def _dot(a, b):
    return jnp.dot(a, b, preferred_element_type=f32)


def _a_ops(a11, a12, a21, a22):
    return (a11 + a22, a21 + a22, a11, a22, a11 + a12, a21 - a11, a12 - a22)


def _b_ops(b11, b12, b21, b22):
    return (b11 + b22, b11, b12 - b22, b21 - b11, b22, b11 + b12, b21 + b22)


def _c_blocks(m):
    c11 = m[0] + m[3] - m[4] + m[6]
    c12 = m[2] + m[4]
    c21 = m[1] + m[3]
    c22 = m[0] - m[1] + m[2] + m[5]
    return c11, c12, c21, c22


def _chunks(n, w):
    out = []
    o = 0
    while o < n:
        e = min(n, o + w)
        out.append((o, e))
        o = e
    return out


def _gate(x, dep):
    if dep is None:
        return x
    if x.shape[0] == 8:
        return x | dep
    return jnp.concatenate([x[0:8] | dep, x[8:]], axis=0)


def _ld(ref, t, lo, hi):
    return pltpu.bitcast(ref[t, :, lo:hi], bf16)


def _st(ref, t, col0, row0, val):
    n, w = val.shape
    if isinstance(row0, int):
        rows = slice(row0 // 2, (row0 + n) // 2)
    else:
        rows = pl.ds(pl.multiple_of(row0 // 2, 8), n // 2)
    if isinstance(col0, int):
        cols = slice(col0, col0 + w)
    else:
        cols = pl.ds(pl.multiple_of(col0, 128), w)
    pk = pltpu.bitcast(val, jnp.uint32)
    ref[t, rows, cols] = pk
    return pk


def _pk(e, o):
    return pltpu.bitcast(pltpu.pack_elementwise([e, o], packed_dtype=bf16), u32)


def _unpk(u, idx):
    return pltpu.unpack_elementwise(u, index=idx, packed_dtype=bf16, unpacked_dtype=f32)


def _ld_eo(ref, r, c0, c1):
    return jnp.concatenate(
        [jnp.concatenate([ref[c, pl.ds(r, 8, stride=2), :], ref[c, pl.ds(r + 1, 8, stride=2), :]], axis=0)
         for c in range(c0, c1)], axis=1)


def _st_eo(ref, t, col0, row0, val):
    pk = _pk(val[0:8], val[8:16])
    rows = slice(row0 // 2, row0 // 2 + 8) if isinstance(row0, int) else pl.ds(pl.multiple_of(row0 // 2, 8), 8)
    ref[t, rows, col0:col0 + val.shape[1]] = pk
    return pk


def _or_all(vals):
    parts = []
    for v in vals:
        for r in range(0, v.shape[0], 8):
            for c in range(0, v.shape[1], 128):
                parts.append(v[r:r + 8, c:c + 128])
    while len(parts) > 1:
        parts = [parts[i] | parts[i + 1] if i + 1 < len(parts) else parts[i] for i in range(0, len(parts), 2)]
    return parts[0]


def _gate_cols(w, deps):
    nk, nn = w.shape[0] // 64, w.shape[1] // 128
    tiles = [(k, j) for j in range(nn) for k in range(nk)]
    at = {tiles[(q * len(tiles)) // len(deps)]: d for q, d in enumerate(deps) if d is not None}
    parts = []
    for k in range(nk):
        if any((k, j) in at for j in range(nn)):
            top = [w[64 * k:64 * k + 8, j * 128:(j + 1) * 128] for j in range(nn)]
            top = [x | at[k, j] if (k, j) in at else x for j, x in enumerate(top)]
            parts += [top[0] if nn == 1 else jnp.concatenate(top, axis=1), w[64 * k + 8:64 * k + 64]]
        else:
            parts.append(w[64 * k:64 * k + 64])
    return pltpu.bitcast(jnp.concatenate(parts, axis=0) if at else w, bf16)


def _stat_dep(x):
    b = pltpu.bitcast(jnp.broadcast_to(x, (16, 128)), u32)
    return b[0:8] | b[8:16]


def _kernel(zero_ref, q_hbm, k_hbm, v_hbm, sk_hbm, h_hbm, dd_hbm, win_hbm, wsp_hbm, bsp_hbm, wout_hbm,
            fwd_hbm, inv_hbm,
            out_hbm,
            kbuf, vbuf, hbuf, qbuf, win_raw, win_s, wsp_raw, wout_raw, wout_s,
            ybuf, xa, xb, z1buf, z2ops, zs, a0, a1, ws0, pa, bcol, obuf,
            kf, spA, spB, wscA, wscB, cpar,
            sk_ref, dd_ref, bsp_ref, fwd_ref, inv_ref,
            sem_kvh, sem_win, sem_misc, sem_out, sem_q0, sem_small):

    def kvh_copies(c):
        cols = pl.ds(pl.multiple_of(c * 128, 128), 128)
        return (
            pltpu.make_async_copy(k_hbm.at[:, cols], kbuf.at[c], sem_kvh.at[c]),
            pltpu.make_async_copy(v_hbm.at[:, cols], vbuf.at[c], sem_kvh.at[c]),
            pltpu.make_async_copy(h_hbm.at[c], hbuf.at[c], sem_kvh.at[c]),
        )

    def win_copies(c):
        r1 = pl.ds(pl.multiple_of(c * WR, WR), WR)
        r2 = pl.ds(pl.multiple_of(D2 + c * WR, WR), WR)
        return (
            pltpu.make_async_copy(win_hbm.at[r1, :], win_raw.at[r1, :], sem_win.at[c]),
            pltpu.make_async_copy(win_hbm.at[r2, :], win_raw.at[r2, :], sem_win.at[c]),
        )

    QS = 3 * TM
    q_copy0 = pltpu.make_async_copy(q_hbm.at[0:TM, :], qbuf.at[0:TM, :], sem_misc.at[0])
    q_copy0b = pltpu.make_async_copy(q_hbm.at[TM:QS, :], qbuf.at[TM:QS, :], sem_misc.at[4])
    q_copy1 = pltpu.make_async_copy(q_hbm.at[QS:S, :], qbuf.at[QS:S, :], sem_misc.at[3])
    wout_copy = pltpu.make_async_copy(wout_hbm, wout_raw, sem_misc.at[1])
    wsp_copy = pltpu.make_async_copy(wsp_hbm, wsp_raw, sem_misc.at[2])

    def start_all(cps):
        for cp in cps:
            cp.start()

    def wait_all(cps):
        for cp in cps:
            cp.wait()

    def kvh0_copies(it):
        rows = pl.ds(pl.multiple_of(it * (S // 4), S // 4), S // 4)
        return (
            pltpu.make_async_copy(k_hbm.at[rows, 0:128], kbuf.at[0, rows, :], sem_q0.at[it]),
            pltpu.make_async_copy(v_hbm.at[rows, 0:128], vbuf.at[0, rows, :], sem_q0.at[it]),
            pltpu.make_async_copy(h_hbm.at[0, :, rows], hbuf.at[0, :, rows], sem_q0.at[it]),
        )

    small0 = (
        pltpu.make_async_copy(sk_hbm, sk_ref, sem_small.at[0]),
        pltpu.make_async_copy(dd_hbm, dd_ref, sem_small.at[0]),
    )
    fwd_copy = pltpu.make_async_copy(fwd_hbm, fwd_ref.at[0:2], sem_small.at[1])
    small2 = (
        pltpu.make_async_copy(inv_hbm, inv_ref.at[0:2], sem_small.at[2]),
        pltpu.make_async_copy(bsp_hbm, bsp_ref, sem_small.at[2]),
    )

    start_all(small0)
    fwd_copy.start()
    for it in range(NQ0):
        start_all(kvh0_copies(it))
    wait_all(small0)
    fwd_copy.wait()
    for it in range(NQ0, 4):
        start_all(kvh0_copies(it))
    start_all(small2)

    sign = jnp.uint32(0x80008000)
    fwd_ref[2:4] = fwd_ref[0:2] ^ sign
    skf = sk_ref[...].astype(f32)
    ddf = dd_ref[...].astype(f32)
    for c in range(NB):
        cpar[c, 0:KS, :] = skf[:, c * 128:(c + 1) * 128]
        cpar[c, KS:KS + 1, :] = ddf[c:c + 1, :]

    def win_presum(c, it, dep):
        RG = 32
        g, half, cb = it // 14, (it // 7) % 2, it % 7
        r = pl.multiple_of(c * WR + g * RG, RG)
        r2 = pl.multiple_of(D2 + c * WR + g * RG, RG)
        o = half * FH + cb * 128
        b11 = pltpu.bitcast(win_raw[pl.ds(r, RG), o:o + 128], u32)
        b12 = pltpu.bitcast(win_raw[pl.ds(r, RG), o + FQ:o + FQ + 128], u32)
        b21 = pltpu.bitcast(win_raw[pl.ds(r2, RG), o:o + 128], u32)
        b22 = pltpu.bitcast(win_raw[pl.ds(r2, RG), o + FQ:o + FQ + 128], u32)
        raw = [_gate(x, dep) for x in (b11, b12, b21, b22)]
        ev = _b_ops(*[_unpk(x, 0) for x in raw])
        od = _b_ops(*[_unpk(x, 1) for x in raw])
        col = half * FQ + cb * 128
        rows = pl.ds(pl.multiple_of(c * (WR // 2) + g * (RG // 2), RG // 2), RG // 2)
        for t in range(7):
            win_s[t, rows, col:col + 128] = _pk(ev[t], od[t]) if t in SUMS else raw[t - 1]

    zsc = [zero_ref[g] for g in range(NC // PG)]
    zmask = jnp.full((8, 128), zsc[0], jnp.int32).astype(u32)

    def conv_stage(c, par, do_prod, do_fwd, do_inv, chunks=range(NC), a0=0, pre=(), mid=None, own=False):
        sp_cur, sp_nxt = (spA, spB) if par == 0 else (spB, spA)
        ws_cur, ws_prv = (wscA, wscB) if par == 0 else (wscB, wscA)
        cn, cp = c + 1, c - 1

        def crow(a, off=0, n=C):
            if isinstance(a0, int):
                return slice((a0 + a) * n + off, (a0 + a + 1) * n + off)
            return pl.ds(pl.multiple_of(a0 * n, n) + (a * n + off), n)

        fin = []

        def inv(a, dep, cur=False):
            wv = (ws_cur if cur else ws_prv)[a0 + a]
            wv = jnp.concatenate([_gate(wv[:C // 2], dep), _gate(wv[C // 2:], dep)], axis=0)
            y = _dot(pltpu.bitcast(inv_ref[a % 4], bf16), pltpu.bitcast(wv, bf16))
            ybuf[c if cur else cp, crow(a), :] = y
            fin.append(pltpu.bitcast(y[C - 8:C], u32))

        def hf(a, dep):
            hv = hbuf[cn, :, crow(a)]
            if dep is not None:
                hv = pltpu.bitcast(_gate(pltpu.bitcast(hv, u32), dep), bf16)
            hj = jax.lax.dot_general(pltpu.bitcast(fwd_ref[a % 4], bf16), hv,
                                     (((1,), (1,)), ((), ())), preferred_element_type=f32)
            if a == 0:
                dd = cpar[cn, KS:KS + 1, :]
                if not isinstance(a0, int):
                    dd = jnp.where(a0 == 0, dd, 0.0)
            for p in range(C // 8):
                re = hj[16 * p:16 * p + 8]
                im = hj[16 * p + 8:16 * p + 16]
                if a == 0:
                    re = re + dd
                sp_nxt[3, a0 + a, 8 * p:8 * p + 8, :] = re
                sp_nxt[4, a0 + a, 8 * p:8 * p + 8, :] = im - re
                sp_nxt[5, a0 + a, 8 * p:8 * p + 8, :] = im + re
            fin.append(pltpu.bitcast(im, u32))

        def uf(a, dep):
            w = [cpar[cn, t:t + 1, :] for t in range(KS)]
            k0 = pltpu.bitcast(kbuf[cn, crow(a), :], u32)
            kf[crow(a, 8, C // 2), :] = k0
            k1 = kf[crow(a, 7, C // 2), :]
            ke, ko, ke1, ko1 = _unpk(k0, 0), _unpk(k0, 1), _unpk(k1, 0), _unpk(k1, 1)
            ko2 = _unpk(kf[crow(a, 6, C // 2), :], 1)
            vw = pltpu.bitcast(vbuf[cn, crow(a), :], u32)
            kse = w[0] * ke + w[1] * ko1 + w[2] * ke1 + w[3] * ko2
            kso = w[0] * ko + w[1] * ke + w[2] * ko1 + w[3] * ke1
            kv = _gate(_pk(kse * _unpk(vw, 0), kso * _unpk(vw, 1)), dep)
            u = _dot(pltpu.bitcast(fwd_ref[a % 4], bf16), pltpu.bitcast(kv, bf16))
            for p in range(C // 8):
                re = u[16 * p:16 * p + 8]
                im = u[16 * p + 8:16 * p + 16]
                sp_nxt[0, a0 + a, 8 * p:8 * p + 8, :] = im + re
                sp_nxt[1, a0 + a, 8 * p:8 * p + 8, :] = re
                sp_nxt[2, a0 + a, 8 * p:8 * p + 8, :] = im
            fin.append(pltpu.bitcast(im, u32))

        prev = {}

        def pgroup(p, g, dep):
            rows = pl.ds(pl.multiple_of(p * 8 + zsc[g] * 8, 8), 8)
            outs = range(g * PG, (g + 1) * PG)
            acc, hw = {}, {}
            for j in range((g + 1) * PG):
                uu = [sp_cur[k, j, rows, :] for k in range(3)]
                if j == 0 and dep is not None:
                    uu = [pltpu.bitcast(_gate(pltpu.bitcast(x, u32), dep), f32) for x in uu]
                for a in outs:
                    l = a - j
                    if l < 0:
                        continue
                    if l not in hw:
                        hw[l] = [sp_cur[3 + k, l, rows, :] for k in range(3)]
                    for k in range(3):
                        pr = hw[l][k] * uu[k]
                        acc[a, k] = pr if (a, k) not in acc else acc[a, k] + pr
            d = None
            for a in outs:
                re = acc[a, 0] - acc[a, 2]
                im = acc[a, 0] + acc[a, 1]
                if a == 0:
                    wr, wi = re, im
                else:
                    wr, wi = re + prev[p][0], im + prev[p][1]
                prev[p] = (re, im)
                pk = pltpu.bitcast(pltpu.pack_elementwise([wr, wi], packed_dtype=bf16), u32)
                ws_cur[a, p * 8:p * 8 + 8, :] = pk
                if a % 2 == 1:
                    d = pk if d is None else d | pk
            return d & zmask

        dots = []
        for a in chunks:
            if do_fwd:
                dots += [(uf, a), (hf, a)]
            if do_inv:
                dots += [(inv, a)]
            for cw in pre:
                dots += [(lambda it, dep, cw=cw: win_presum(cw, it, dep), it)
                         for it in range(a * 28 // NC, (a + 1) * 28 // NC)]
        cost = [PC if fn not in (uf, hf, inv) else 256 for fn, _ in dots]
        pos = (np.cumsum(cost) - cost - LEAD * 256) / sum(cost) * STR
        nd = len(dots)
        if not do_prod:
            for fn, a in dots:
                fn(a, None)
            return
        ng = NC // PG
        order = [(p, g) for p in range(C // 8) for g in range(ng)]
        if own:
            order = [x for x in order if x[1] < ng - 1] + [x for x in order if x[1] == ng - 1]
        wts = [sum(a + 1 for a in range(g * PG, (g + 1) * PG)) for _, g in order]
        cum = np.cumsum(wts) / sum(wts)
        if own:
            ca = cum[(C // 8) * (ng - 1) - 1]
            n = NC - PG
            dots += [(lambda a, dep: inv(a, dep, True), a) for a in range(n)]
            pos = list(pos * ca / STR) + [ca + k * (OS - ca) / n for k in range(n)]
            nd = len(dots)
        i0 = 0 if mid is None else P0 * ng
        base = 0.0 if i0 == 0 else cum[i0 - 1]
        cum = (cum - base) / (1.0 - base)
        d = 0
        dep = None
        i = 0
        for p, g in order:
            if i == i0:
                if mid is not None:
                    mid()
                while d < nd and pos[d] <= 0:
                    dots[d][0](dots[d][1], None)
                    d += 1
            if i == RQ:
                assert d == nd
                dep = dep | (_or_all(fin[-RN:]) & zmask)
            dep = pgroup(p, g, dep)
            while i >= i0 and d < nd and pos[d] <= cum[i]:
                dots[d][0](dots[d][1], dep)
                d += 1
            i += 1

    kf[0:8, :] = jnp.zeros((8, 128), u32)

    with jax.named_scope('conv'):
        def first_body(it, carry):
            wait_all(kvh0_copies(it))

            @pl.when(it == K1)
            def _():
                start_all(kvh_copies(1))
            conv_stage(-1, 1, False, True, False, range(4), it * 4)
            return carry
        jax.lax.fori_loop(0, NC // 4, first_body, 0)
        xb[:, 0:TM, :] = jnp.zeros((NB, TM, 128), f32)
        wait_all(small2)
        inv_ref[2:4] = inv_ref[0:2] ^ sign
        for r in range(S // 128):
            row = bsp_ref[r:r + 1, :].astype(f32)
            bcol[r * 128:(r + 1) * 128, :] = 0.5 * jnp.broadcast_to(row, (128, 128)).T

        def mid0():
            cps = kvh_copies(1)
            wait_all(cps[:2])
            start_all(kvh_copies(2))
            wait_all(cps[2:])
        conv_stage(0, 0, True, True, False, mid=mid0)

        def conv_body(ii, carry):
            for e in range(2):
                c = 2 * ii + 1 + e
                cps = kvh_copies(c + 1)
                if e == 0:
                    @pl.when(c >= 2)
                    def _():
                        wait_all(win_copies(c - 2))
                    wait_all(cps[:2])
                    start_all(kvh_copies(c + 2))
                    start_all(win_copies(c - 1))
                    cw = jnp.where(c >= 2, c - 2, NB - 1)
                else:
                    wait_all(win_copies(c - 2))
                    wait_all(cps[:2])

                    @pl.when(c + 2 < NB)
                    def _():
                        start_all(kvh_copies(c + 2))

                    @pl.when(c + 2 == NB)
                    def _():
                        start_all(win_copies(c))
                        q_copy0.start()
                    start_all(win_copies(c - 1))
                    cw = c - 2
                wait_all(cps[2:])
                conv_stage(c, 1 - e, True, True, True, pre=(cw,))
            return carry
        jax.lax.fori_loop(0, NB // 2 - 1, conv_body, 0)
        wait_all(win_copies(NB - 3))
        start_all(win_copies(NB - 1))
        q_copy0b.start()
        wait_all(win_copies(NB - 2))
        conv_stage(NB - 1, 1, True, False, True, pre=(NB - 3, NB - 2), own=True)

    q_copy0.wait()
    wait_all(win_copies(NB - 1))

    conv_stage(NB, 0, False, False, True, range(NC - PG, NC))
    for it in range(28):
        win_presum(NB - 1, it, None)

    def wout_b(t, lo, hi):
        if t == 1:
            return pltpu.bitcast(wout_raw[0:FQ, lo:hi], u32)
        if t == 4:
            return pltpu.bitcast(wout_raw[FQ:FH, D2 + lo:D2 + hi], u32)
        return wout_s[SUMS.index(t), :, lo:hi]

    RG = 16
    NG = H // RG

    def a_buf(ref):
        return (lambda t: _ld(ref, t, 0, D2)), (lambda t, lo, g, val: _st_eo(ref, t, lo, g * RG, val))

    def prologue_steps(i, src, a_st, groups=range(NG), idst=None):
        for g in groups:
            st = []
            for hh in range(2):
                r = pl.multiple_of(i * TM + hh * H + g * RG, RG)
                rd = r if idst is None else pl.multiple_of(idst * TM + hh * H + g * RG, RG)
                if src is qbuf:
                    xq = pltpu.bitcast(src[pl.ds(r, RG), :], u32)
                    x = jnp.concatenate([_unpk(xq, 0), _unpk(xq, 1)], axis=0)
                else:
                    x = _ld_eo(src, r, 0, NB)
                x1 = x + _ln(x) * _ld_eo(ybuf, r, 0, NB)
                for c in range(NB):
                    xa[c, pl.ds(rd, 8, stride=2), :] = x1[0:8, c * 128:(c + 1) * 128]
                    xa[c, pl.ds(rd + 1, 8, stride=2), :] = x1[8:16, c * 128:(c + 1) * 128]
                m = jnp.mean(x1, axis=-1, keepdims=True)
                xc = x1 - m
                rs = jax.lax.rsqrt(jnp.mean(xc * xc, axis=-1, keepdims=True) + EPS)
                st.append((pl.multiple_of((i if idst is None else idst) * TM + hh * H + g * RG + zsc[1] * RG, RG), m, rs))
                yield _stat_dep(rs) & zmask
            for (lo, hi) in _chunks(D2, PW):
                q4 = []
                for hh in range(2):
                    rw, m, rs = st[hh]
                    for o in (0, D2):
                        q4.append((_ld_eo(xa, rw, (o + lo) // 128, (o + hi) // 128) - m) * rs)
                ops = _a_ops(*q4)
                yield _or_all([a_st(t, lo, g, ops[t]) for t in range(7)]) & zmask

    def prologue0(a_st):
        def row(j, k):
            return pl.multiple_of(j * RG + zsc[k] * RG, RG)

        def ldq(j, k):
            xq = pltpu.bitcast(qbuf[pl.ds(row(j, k), RG), :], u32)
            return jnp.concatenate([_unpk(xq, 0), _unpk(xq, 1)], axis=0)

        def rstd(xc):
            return jax.lax.rsqrt(jnp.mean(xc * xc, axis=-1, keepdims=True) + EPS)
        js = range(2 * NG)
        m1 = [jnp.mean(ldq(j, 0), axis=-1, keepdims=True) for j in js]
        r1 = [rstd(ldq(j, 1) - m1[j]) for j in js]
        m2 = []
        for j in js:
            x = ldq(j, 2)
            x1 = x + (x - m1[j]) * r1[j] * _ld_eo(ybuf, j * RG, 0, NB)
            for c in range(NB):
                xa[c, pl.ds(j * RG, 8, stride=2), :] = x1[0:8, c * 128:(c + 1) * 128]
                xa[c, pl.ds(j * RG + 1, 8, stride=2), :] = x1[8:16, c * 128:(c + 1) * 128]
            m2.append(jnp.mean(x1, axis=-1, keepdims=True))
        r2 = [rstd(_ld_eo(xa, row(j, 0), 0, NB) - m2[j]) for j in js]
        for g in range(NG):
            for (lo, hi) in _chunks(D2, PW):
                q4 = [(_ld_eo(xa, row(j, 1), (o + lo) // 128, (o + hi) // 128) - m2[j]) * r2[j]
                      for j in (g, NG + g) for o in (0, D2)]
                ops = _a_ops(*q4)
                for t in range(7):
                    a_st(t, lo, g, ops[t])

    PS = 2 + len(_chunks(D2, PW))

    def z2_steps(i, fence):
        for g in range(NG):
            rq = pl.multiple_of(i * H + g * RG, RG)
            fence()
            st = []
            for hh in range(2):
                def row(k):
                    return pl.multiple_of(hh * H + g * RG + zsc[k] * RG, RG)
                m = jnp.mean(_ld_eo(zs, row(0), 0, FH // 128), axis=-1, keepdims=True)
                xc = _ld_eo(zs, row(1), 0, FH // 128) - m
                v = jnp.mean(xc * xc, axis=-1, keepdims=True)
                st.append((row(2), m, 0.5 * jax.lax.rsqrt(v + 4.0 * EPS)))
            yield (_stat_dep(st[0][2]) | _stat_dep(st[1][2])) & zmask
            for (lo, hi) in _chunks(FQ, ZW):
                q4 = []
                for hh in range(2):
                    rw, m, rs = st[hh]
                    for o in (0, FQ):
                        q4.append((_ld_eo(zs, rw, (o + lo) // 128, (o + hi) // 128) - m) * rs)
                ops = _b_ops(*q4)
                yield _or_all([_st_eo(z2ops, t, lo, rq, ops[t]) for t in range(7)]) & zmask

    def spread(nsteps, first, last, sl):
        lo, hi = first * sl, (last + 1) * sl - 1
        return [lo + (k * (hi - lo)) // max(nsteps - 1, 1) for k in range(nsteps)]

    def anchors(steps, slots):
        state = [0]

        def take(n):
            deps = []
            for _ in range(n):
                d = None
                while slots and slots[0] <= state[0]:
                    slots.pop(0)
                    dn = next(steps)
                    d = dn if d is None else d | dn
                deps.append(d)
                state[0] += 1
            return deps
        return take

    def wout_steps():
        for g in range(FQ // WRB):
            for (lo, hi) in _chunks(D2, WC):
                raw = [pltpu.bitcast(wout_raw[r0 + g * WRB:r0 + (g + 1) * WRB, c0 + lo:c0 + hi], u32)
                       for r0 in (0, FQ) for c0 in (0, D2)]
                ev = _b_ops(*[_unpk(x, 0) for x in raw])
                od = _b_ops(*[_unpk(x, 1) for x in raw])
                pks = [_pk(ev[t], od[t]) for t in SUMS]
                for k in range(5):
                    wout_s[k, g * WRB // 2:(g + 1) * WRB // 2, lo:hi] = pks[k]
                yield _or_all(pks) & zmask

    def mm1(i, a_ld, psteps, nps):
        hist = []

        def fence():
            if len(hist) >= ZK:
                zs[FH // 128 + zsc[0], 0:8, :] = hist[-ZK][0:8, 0:128]

        def half(off, steps, slots, store):
            take = anchors(steps, slots)
            for (lo, hi) in _chunks(FQ, TN):
                m = []
                for t in range(7):
                    deps = take((hi - lo) // 128 * SL1)
                    m.append(_dot(a_ld(t), _gate_cols(win_s[t, :, off + lo:off + hi], deps)))
                    hist.append(m[-1])
                c11, c12, c21, c22 = _c_blocks(m)
                store(0, lo, hi, _gelu(c11))
                store(0, FQ + lo, FQ + hi, _gelu(c12))
                store(1, lo, hi, _gelu(c21))
                store(1, FQ + lo, FQ + hi, _gelu(c22))

        def store_z2(hh, lo, hi, val):
            for c in range(lo // 128, hi // 128):
                zs[c, hh * H:(hh + 1) * H, :] = val[:, c * 128 - lo:(c + 1) * 128 - lo]

        def store_z1(hh, lo, hi, val):
            z1buf[pl.ds(pl.multiple_of(i * H + hh * (H // 2), H // 2), H // 2), lo:hi] = _pk(val[:H // 2], val[H // 2:])

        half(FQ, psteps, spread(nps, PA[0], PA[1], SL1), store_z2)
        del hist[:]
        half(0, z2_steps(i, fence), spread(NG * (1 + len(_chunks(FQ, ZW))), ZA[0], ZA[1], SL1), store_z1)

    def ws_steps(i, ws_ref):
        G = BG
        for g in range(H // G):
            r1 = pl.ds(pl.multiple_of(i * TM + g * G, G), G)
            r2 = pl.ds(pl.multiple_of(i * TM + H + g * G, G), G)
            for t in range(NT):
                raw = [pltpu.bitcast(wsp_raw[rr, c0:c0 + H], u32)
                       for rr in (r1, r2) for c0 in (t * TM, t * TM + H)]
                ev = _a_ops(*[_unpk(x, 0) for x in raw])
                od = _a_ops(*[_unpk(x, 1) for x in raw])
                vals = [raw[0] if u == 2 else raw[3] if u == 3 else _pk(ev[u], od[u]) for u in range(7)]
                for u in range(7):
                    ws_ref[u + zsc[0], g * G // 2:(g + 1) * G // 2, t * H:(t + 1) * H] = vals[u]
                yield _or_all([vals[u] for u in (0, 1, 4, 5, 6)]) & zmask

    def mm23(i, inext, ws_ref, src, store, take, done=None):
        r = pl.multiple_of(i * TM, TM)
        for (lo, hi) in _chunks(FQ, TN):
            wdt = hi - lo
            m = [_dot(_ld(ws_ref, t, 0, S // 2), _gate_cols(z2ops[t, :, lo:hi], take(wdt // 128 * SL2)))
                 for t in range(7)]
            c11, c12, c21, c22 = _c_blocks(m)
            b1 = jnp.concatenate([bcol[pl.ds(r, H), :]] * (wdt // 128), axis=1)
            b2 = jnp.concatenate([bcol[pl.ds(r + H, H), :]] * (wdt // 128), axis=1)
            def z1(hh, c0):
                w = z1buf[pl.ds(pl.multiple_of(i * H + hh * (H // 2), H // 2), H // 2), c0:c0 + wdt]
                return jnp.concatenate([_unpk(w, 0), _unpk(w, 1)], axis=0)
            p11 = z1(0, lo) * (c11 + b1)
            p12 = z1(0, FQ + lo) * (c12 + b1)
            p21 = z1(1, lo) * (c21 + b2)
            p22 = z1(1, FQ + lo) * (c22 + b2)
            ops = _a_ops(p11, p12, p21, p22)
            for t in range(7):
                _st(pa, t, lo, 0, ops[t].astype(bf16))
        take3 = anchors(ws_steps(inext, ws_ref), spread(H // BG * NT, BA[0], BA[1], SL3))
        for (lo, hi) in _chunks(D2, TN):
            m = [_dot(_ld(pa, t, 0, FQ), _gate_cols(wout_b(t, lo, hi), take3((hi - lo) // 128 * SL3)))
                 for t in range(7)]
            c11, c12, c21, c22 = _c_blocks(m)
            def res(hh, c0):
                return jnp.concatenate([src[c, pl.ds(r + hh * H, H), :]
                                        for c in range(c0 // 128, (c0 + hi - lo) // 128)], axis=1)
            store(0, lo, hi, res(0, lo) + c11)
            store(0, D2 + lo, D2 + hi, res(0, D2 + lo) + c12)
            store(1, lo, hi, res(1, lo) + c21)
            store(1, D2 + lo, D2 + hi, res(1, D2 + lo) + c22)
            if done is not None:
                done(lo)

    def out_copy(i, slot, los=range(0, D2, TN)):
        rows = pl.ds(pl.multiple_of(i * TM, TM), TM)
        return [pltpu.make_async_copy(obuf.at[slot, :, c0:c0 + TN], out_hbm.at[rows, c0:c0 + TN], sem_out.at[slot])
                for lo in los for c0 in (lo, D2 + lo)]

    def merge(steps_a, slots_a, steps_b, slots_b):
        order = sorted([(q, 0) for q in slots_a] + [(q, 1) for q in slots_b])

        def gen():
            for _, w in order:
                yield next(steps_b if w else steps_a)
        return anchors(gen(), [q for q, _ in order])

    (ld0, st0), (ld1, st1) = a_buf(a0), a_buf(a1)
    prologue0(st0)
    q_copy1.start()
    q_copy0b.wait()

    for layer in range(2):
        def p1_body(ii, carry, layer=layer):
            i = 2 * ii
            if layer == 0:
                @pl.when(ii == 1)
                def _():
                    q_copy1.wait()
                    wout_copy.start()
                    wsp_copy.start()
            src = qbuf if layer == 0 else xb
            mm1(i, ld0, prologue_steps(i + 1, src, st1), NG * PS)
            mm1(i + 1, ld1, prologue_steps(jnp.minimum(i + 2, NT - 1), src, st0), NG * PS)
            return carry

        with jax.named_scope(f'p1_{layer}'):
            jax.lax.fori_loop(0, NT // 2, p1_body, 0)

        if layer == 0:
            wout_copy.wait()
            wsp_copy.wait()
            for _ in ws_steps(0, ws0):
                pass

        if layer == 0:
            def p2_body(i, carry):
                r = pl.multiple_of(i * TM, TM)

                def store(hh, lo, hi, val):
                    for c in range(lo // 128, hi // 128):
                        xb[c, pl.ds(r + hh * H, H), :] = val[:, c * 128 - lo:(c + 1) * 128 - lo]
                g0 = 2 * jnp.clip(i - 1, 0, NG // 2 - 1)
                take = merge(wout_steps(), spread(FQ // WRB * (D2 // WC), WA[0], WA[1], SL2),
                             prologue_steps(0, xb, st0, (g0, g0 + 1), jnp.where(i == 0, NT, 0)),
                             spread(2 * PS, QA[0], QA[1], SL2))
                mm23(i, (i + 1) % NT, ws0, xa, store, take)
                return carry
            with jax.named_scope(f'p2_{layer}'):
                jax.lax.fori_loop(0, NT, p2_body, 0)
        else:
            def p2_body(i, carry):
                slot = i % 2

                def store(hh, lo, hi, val):
                    obuf[slot, hh * H:(hh + 1) * H, lo:hi] = val.astype(bf16)

                @pl.when(i >= 2)
                def _():
                    wait_all(out_copy(i - 2, slot))
                mm23(i, (i + 1) % NT, ws0, xa, store, anchors(None, []),
                     lambda lo: start_all(out_copy(i, slot, (lo,))))
                return carry
            with jax.named_scope(f'p2_{layer}'):
                jax.lax.fori_loop(0, NT, p2_body, 0)
            wait_all(out_copy(NT - 2, 0))
            wait_all(out_copy(NT - 1, 1))


@jax.jit
def pallas_interleave_layers__ssm_conv_h3__mixer_gmlp__prompt_kernel(
    A_q: jax.Array,
    A_k: jax.Array,
    A_v: jax.Array,
    A_shift_k: jax.Array,
    A_ssm_k: jax.Array,
    A_ssm_D: jax.Array,
    B_x: jax.Array,
    B_w_in: jax.Array,
    B_w_sp: jax.Array,
    B_b_sp: jax.Array,
    B_w_out: jax.Array,
):
    fwd_np, inv_np = _dft_mats()
    fwd = jnp.asarray(fwd_np)
    inv = jnp.asarray(inv_np)
    zero = jnp.asarray(np.zeros((8,), np.int32))

    any_spec = pl.BlockSpec(memory_space=pl.ANY)
    smem_spec = pl.BlockSpec(memory_space=pltpu.SMEM)

    scratch = [
        pltpu.VMEM((NB, S, 128), bf16),
        pltpu.VMEM((NB, S, 128), bf16),
        pltpu.VMEM((NB, 128, S), bf16),
        pltpu.VMEM((S, D), bf16),
        pltpu.VMEM((D, F), bf16),
        pltpu.VMEM((7, D2 // 2, FH), u32),
        pltpu.VMEM((S, S), bf16),
        pltpu.VMEM((FH, D), bf16),
        pltpu.VMEM((5, FQ // 2, D2), u32),
        pltpu.VMEM((NB, S, 128), f32),
        pltpu.VMEM((NB, S + TM, 128), f32),
        pltpu.VMEM((NB, S, 128), f32),
        pltpu.VMEM((S // 2, FH), u32),
        pltpu.VMEM((7, S // 4, FQ), u32),
        pltpu.VMEM((FH // 128 + 1, TM, 128), f32),
        pltpu.VMEM((7, H // 2, D2), u32),
        pltpu.VMEM((7, H // 2, D2), u32),
        pltpu.VMEM((7, H // 2, S // 2), u32),
        pltpu.VMEM((7, H // 2, FQ), u32),
        pltpu.VMEM((S, 128), f32),
        pltpu.VMEM((2, TM, D), bf16),
        pltpu.VMEM((S // 2 + 8, 128), u32),
        pltpu.VMEM((6, NC + 1, CP, 128), f32),
        pltpu.VMEM((6, NC + 1, CP, 128), f32),
        pltpu.VMEM((NC, C, 128), u32),
        pltpu.VMEM((NC, C, 128), u32),
        pltpu.VMEM((NB, 8, 128), f32),
        pltpu.VMEM((KS, D), bf16),
        pltpu.VMEM((NB, 128), bf16),
        pltpu.VMEM((S // 128, 128), bf16),
        pltpu.VMEM((4, C, C), u32),
        pltpu.VMEM((4, C // 2, 2 * C), u32),
        pltpu.SemaphoreType.DMA((NB,)),
        pltpu.SemaphoreType.DMA((NB,)),
        pltpu.SemaphoreType.DMA((5,)),
        pltpu.SemaphoreType.DMA((2,)),
        pltpu.SemaphoreType.DMA((4,)),
        pltpu.SemaphoreType.DMA((3,)),
    ]

    out = pl.pallas_call(
        _kernel,
        in_specs=[smem_spec] + [any_spec] * 12,
        out_specs=any_spec,
        out_shape=jax.ShapeDtypeStruct((S, D), bf16),
        scratch_shapes=scratch,
        compiler_params=pltpu.CompilerParams(vmem_limit_bytes=127 * 1024 * 1024, disable_bounds_checks=True),
    )(
        zero,
        A_q.reshape(S, D), A_k.reshape(S, D), A_v.reshape(S, D),
        A_shift_k.T, A_ssm_k.reshape(NB, 128, S), A_ssm_D.reshape(NB, 128),
        B_w_in, B_w_sp, B_b_sp.reshape(S // 128, 128), B_w_out,
        fwd, inv,
    )
    return out.reshape(1, S, D)
```

```python
import numpy as np
import jax
import jax.numpy as jnp
import jax.experimental.pallas as pl
import jax.experimental.pallas.tpu as pltpu

f32 = jnp.float32
bf16 = jnp.bfloat16
u32 = jnp.uint32

S = 2048
D = 1024
F = 3584
FH = F // 2
FQ = FH // 2
D2 = D // 2
C = 128
NC = S // C
NB = D // 128
TM = 256
H = TM // 2
NT = S // TM
EPS = 1e-5
KS = 4
TN = 256
WR = D2 // NB
PG = 4
CP = C + 8
LEAD, STR, PC = 3, 0.85, 50
RQ, RN, OS, P0 = 62, 3, 0.85, 8
NQ0, K1 = 2, 2
PW = ZW = WC = 256
WRB, BG, ZK = 16, 32, 3
SL1, SL2, SL3 = 2, 8, 7
PA, ZA, QA, WA, BA = (5, 48), (7, 48), (3, 46), (3, 44), (2, 26)
SUMS = (0, 2, 3, 5, 6)


def _pack_rows(m):
    b = m.astype(bf16).view(np.uint16).astype(np.uint32)
    return b[0::2] | (b[1::2] << 16)


def _dft_mats():
    f = np.arange(C, dtype=np.float64)
    b = np.arange(C, dtype=np.float64)
    perm_f = np.concatenate([np.concatenate([np.arange(8 * p, 8 * p + 8), C + np.arange(8 * p, 8 * p + 8)])
                             for p in range(C // 8)])
    perm_i = np.stack([np.arange(C), C + np.arange(C)], axis=1).reshape(-1)
    fwds, invs = [], []
    for a in range(2):
        ang = 2.0 * np.pi * (f[:, None] + 0.5) * (b[None, :] + C * a) / (2 * C)
        fwd = np.concatenate([np.cos(ang), -np.sin(ang)], axis=0)
        inv = (fwd.T / C)[:, perm_i]
        fwds.append(_pack_rows(fwd[perm_f].astype(np.float32)))
        invs.append(_pack_rows(inv.astype(np.float32)))
    return np.stack(fwds), np.stack(invs)


def _ln(x):
    m = jnp.mean(x, axis=-1, keepdims=True)
    xc = x - m
    v = jnp.mean(xc * xc, axis=-1, keepdims=True)
    return xc * jax.lax.rsqrt(v + EPS)


def _gelu(x):
    c0 = 0.7978845608028654
    inner = x * (c0 + (c0 * 0.044715) * (x * x))
    return x + x * jnp.tanh(inner)


def _dot(a, b):
    return jnp.dot(a, b, preferred_element_type=f32)


def _a_ops(a11, a12, a21, a22):
    return (a11 + a22, a21 + a22, a11, a22, a11 + a12, a21 - a11, a12 - a22)


def _b_ops(b11, b12, b21, b22):
    return (b11 + b22, b11, b12 - b22, b21 - b11, b22, b11 + b12, b21 + b22)


def _c_blocks(m):
    c11 = m[0] + m[3] - m[4] + m[6]
    c12 = m[2] + m[4]
    c21 = m[1] + m[3]
    c22 = m[0] - m[1] + m[2] + m[5]
    return c11, c12, c21, c22


def _chunks(n, w):
    out = []
    o = 0
    while o < n:
        e = min(n, o + w)
        out.append((o, e))
        o = e
    return out


def _gate(x, dep):
    if dep is None:
        return x
    if x.shape[0] == 8:
        return x | dep
    return jnp.concatenate([x[0:8] | dep, x[8:]], axis=0)


def _ld(ref, t, lo, hi):
    return pltpu.bitcast(ref[t, :, lo:hi], bf16)


def _st(ref, t, col0, row0, val):
    n, w = val.shape
    if isinstance(row0, int):
        rows = slice(row0 // 2, (row0 + n) // 2)
    else:
        rows = pl.ds(pl.multiple_of(row0 // 2, 8), n // 2)
    if isinstance(col0, int):
        cols = slice(col0, col0 + w)
    else:
        cols = pl.ds(pl.multiple_of(col0, 128), w)
    pk = pltpu.bitcast(val, jnp.uint32)
    ref[t, rows, cols] = pk
    return pk


def _pk(e, o):
    return pltpu.bitcast(pltpu.pack_elementwise([e, o], packed_dtype=bf16), u32)


def _unpk(u, idx):
    return pltpu.unpack_elementwise(u, index=idx, packed_dtype=bf16, unpacked_dtype=f32)


def _ld_eo(ref, r, c0, c1):
    return jnp.concatenate(
        [jnp.concatenate([ref[c, pl.ds(r, 8, stride=2), :], ref[c, pl.ds(r + 1, 8, stride=2), :]], axis=0)
         for c in range(c0, c1)], axis=1)


def _st_eo(ref, t, col0, row0, val):
    pk = _pk(val[0:8], val[8:16])
    rows = slice(row0 // 2, row0 // 2 + 8) if isinstance(row0, int) else pl.ds(pl.multiple_of(row0 // 2, 8), 8)
    ref[t, rows, col0:col0 + val.shape[1]] = pk
    return pk


def _or_all(vals):
    parts = []
    for v in vals:
        for r in range(0, v.shape[0], 8):
            for c in range(0, v.shape[1], 128):
                parts.append(v[r:r + 8, c:c + 128])
    while len(parts) > 1:
        parts = [parts[i] | parts[i + 1] if i + 1 < len(parts) else parts[i] for i in range(0, len(parts), 2)]
    return parts[0]


def _gate_cols(w, deps):
    nk, nn = w.shape[0] // 64, w.shape[1] // 128
    tiles = [(k, j) for j in range(nn) for k in range(nk)]
    at = {tiles[(q * len(tiles)) // len(deps)]: d for q, d in enumerate(deps) if d is not None}
    parts = []
    for k in range(nk):
        if any((k, j) in at for j in range(nn)):
            top = [w[64 * k:64 * k + 8, j * 128:(j + 1) * 128] for j in range(nn)]
            top = [x | at[k, j] if (k, j) in at else x for j, x in enumerate(top)]
            parts += [top[0] if nn == 1 else jnp.concatenate(top, axis=1), w[64 * k + 8:64 * k + 64]]
        else:
            parts.append(w[64 * k:64 * k + 64])
    return pltpu.bitcast(jnp.concatenate(parts, axis=0) if at else w, bf16)


def _stat_dep(x):
    b = pltpu.bitcast(jnp.broadcast_to(x, (16, 128)), u32)
    return b[0:8] | b[8:16]


def _kernel(zero_ref, q_hbm, k_hbm, v_hbm, sk_hbm, h_hbm, dd_hbm, win_hbm, wsp_hbm, bsp_hbm, wout_hbm,
            fwd_hbm, inv_hbm,
            out_hbm,
            kbuf, vbuf, hbuf, qbuf, win_raw, win_s, wsp_raw, wout_raw, wout_s,
            ybuf, xa, xb, z1buf, z2ops, zs, a0, a1, ws0, pa, bcol, obuf,
            kf, spA, spB, wscA, wscB, cpar,
            sk_ref, dd_ref, bsp_ref, fwd_ref, inv_ref,
            sem_kvh, sem_win, sem_misc, sem_out, sem_q0, sem_small):

    def kvh_copies(c):
        cols = pl.ds(pl.multiple_of(c * 128, 128), 128)
        return (
            pltpu.make_async_copy(k_hbm.at[:, cols], kbuf.at[c], sem_kvh.at[c]),
            pltpu.make_async_copy(v_hbm.at[:, cols], vbuf.at[c], sem_kvh.at[c]),
            pltpu.make_async_copy(h_hbm.at[c], hbuf.at[c], sem_kvh.at[c]),
        )

    def win_copies(c):
        r1 = pl.ds(pl.multiple_of(c * WR, WR), WR)
        r2 = pl.ds(pl.multiple_of(D2 + c * WR, WR), WR)
        return (
            pltpu.make_async_copy(win_hbm.at[r1, :], win_raw.at[r1, :], sem_win.at[c]),
            pltpu.make_async_copy(win_hbm.at[r2, :], win_raw.at[r2, :], sem_win.at[c]),
        )

    QS = 3 * TM
    q_copy0 = pltpu.make_async_copy(q_hbm.at[0:TM, :], qbuf.at[0:TM, :], sem_misc.at[0])
    q_copy0b = pltpu.make_async_copy(q_hbm.at[TM:QS, :], qbuf.at[TM:QS, :], sem_misc.at[4])
    q_copy1 = pltpu.make_async_copy(q_hbm.at[QS:S, :], qbuf.at[QS:S, :], sem_misc.at[3])
    wout_copy = pltpu.make_async_copy(wout_hbm, wout_raw, sem_misc.at[1])
    wsp_copy = pltpu.make_async_copy(wsp_hbm, wsp_raw, sem_misc.at[2])

    def start_all(cps):
        for cp in cps:
            cp.start()

    def wait_all(cps):
        for cp in cps:
            cp.wait()

    def kvh0_copies(it):
        rows = pl.ds(pl.multiple_of(it * (S // 4), S // 4), S // 4)
        return (
            pltpu.make_async_copy(k_hbm.at[rows, 0:128], kbuf.at[0, rows, :], sem_q0.at[it]),
            pltpu.make_async_copy(v_hbm.at[rows, 0:128], vbuf.at[0, rows, :], sem_q0.at[it]),
            pltpu.make_async_copy(h_hbm.at[0, :, rows], hbuf.at[0, :, rows], sem_q0.at[it]),
        )

    small0 = (
        pltpu.make_async_copy(sk_hbm, sk_ref, sem_small.at[0]),
        pltpu.make_async_copy(dd_hbm, dd_ref, sem_small.at[0]),
    )
    fwd_copy = pltpu.make_async_copy(fwd_hbm, fwd_ref.at[0:2], sem_small.at[1])
    small2 = (
        pltpu.make_async_copy(inv_hbm, inv_ref.at[0:2], sem_small.at[2]),
        pltpu.make_async_copy(bsp_hbm, bsp_ref, sem_small.at[2]),
    )

    start_all(small0)
    fwd_copy.start()
    for it in range(NQ0):
        start_all(kvh0_copies(it))
    wait_all(small0)
    fwd_copy.wait()
    for it in range(NQ0, 4):
        start_all(kvh0_copies(it))
    start_all(small2)

    sign = jnp.uint32(0x80008000)
    fwd_ref[2:4] = fwd_ref[0:2] ^ sign
    skf = sk_ref[...].astype(f32)
    ddf = dd_ref[...].astype(f32)
    for c in range(NB):
        cpar[c, 0:KS, :] = skf[:, c * 128:(c + 1) * 128]
        cpar[c, KS:KS + 1, :] = ddf[c:c + 1, :]

    def win_presum(c, it, dep):
        RG = 32
        g, half, cb = it // 14, (it // 7) % 2, it % 7
        r = pl.multiple_of(c * WR + g * RG, RG)
        r2 = pl.multiple_of(D2 + c * WR + g * RG, RG)
        o = half * FH + cb * 128
        b11 = pltpu.bitcast(win_raw[pl.ds(r, RG), o:o + 128], u32)
        b12 = pltpu.bitcast(win_raw[pl.ds(r, RG), o + FQ:o + FQ + 128], u32)
        b21 = pltpu.bitcast(win_raw[pl.ds(r2, RG), o:o + 128], u32)
        b22 = pltpu.bitcast(win_raw[pl.ds(r2, RG), o + FQ:o + FQ + 128], u32)
        raw = [_gate(x, dep) for x in (b11, b12, b21, b22)]
        ev = _b_ops(*[_unpk(x, 0) for x in raw])
        od = _b_ops(*[_unpk(x, 1) for x in raw])
        col = half * FQ + cb * 128
        rows = pl.ds(pl.multiple_of(c * (WR // 2) + g * (RG // 2), RG // 2), RG // 2)
        for t in range(7):
            win_s[t, rows, col:col + 128] = _pk(ev[t], od[t]) if t in SUMS else raw[t - 1]

    zsc = [zero_ref[g] for g in range(NC // PG)]
    zmask = jnp.full((8, 128), zsc[0], jnp.int32).astype(u32)

    def conv_stage(c, par, do_prod, do_fwd, do_inv, chunks=range(NC), a0=0, pre=(), mid=None, own=False):
        sp_cur, sp_nxt = (spA, spB) if par == 0 else (spB, spA)
        ws_cur, ws_prv = (wscA, wscB) if par == 0 else (wscB, wscA)
        cn, cp = c + 1, c - 1

        def crow(a, off=0, n=C):
            if isinstance(a0, int):
                return slice((a0 + a) * n + off, (a0 + a + 1) * n + off)
            return pl.ds(pl.multiple_of(a0 * n, n) + (a * n + off), n)

        fin = []

        def inv(a, dep, cur=False):
            wv = (ws_cur if cur else ws_prv)[a0 + a]
            wv = jnp.concatenate([_gate(wv[:C // 2], dep), _gate(wv[C // 2:], dep)], axis=0)
            y = _dot(pltpu.bitcast(inv_ref[a % 4], bf16), pltpu.bitcast(wv, bf16))
            ybuf[c if cur else cp, crow(a), :] = y
            fin.append(pltpu.bitcast(y[C - 8:C], u32))

        def hf(a, dep):
            hv = hbuf[cn, :, crow(a)]
            if dep is not None:
                hv = pltpu.bitcast(_gate(pltpu.bitcast(hv, u32), dep), bf16)
            hj = jax.lax.dot_general(pltpu.bitcast(fwd_ref[a % 4], bf16), hv,
                                     (((1,), (1,)), ((), ())), preferred_element_type=f32)
            if a == 0:
                dd = cpar[cn, KS:KS + 1, :]
                if not isinstance(a0, int):
                    dd = jnp.where(a0 == 0, dd, 0.0)
            for p in range(C // 8):
                re = hj[16 * p:16 * p + 8]
                im = hj[16 * p + 8:16 * p + 16]
                if a == 0:
                    re = re + dd
                sp_nxt[3, a0 + a, 8 * p:8 * p + 8, :] = re
                sp_nxt[4, a0 + a, 8 * p:8 * p + 8, :] = im - re
                sp_nxt[5, a0 + a, 8 * p:8 * p + 8, :] = im + re
            fin.append(pltpu.bitcast(im, u32))

        def uf(a, dep):
            w = [cpar[cn, t:t + 1, :] for t in range(KS)]
            k0 = pltpu.bitcast(kbuf[cn, crow(a), :], u32)
            kf[crow(a, 8, C // 2), :] = k0
            k1 = kf[crow(a, 7, C // 2), :]
            ke, ko, ke1, ko1 = _unpk(k0, 0), _unpk(k0, 1), _unpk(k1, 0), _unpk(k1, 1)
            ko2 = _unpk(kf[crow(a, 6, C // 2), :], 1)
            vw = pltpu.bitcast(vbuf[cn, crow(a), :], u32)
            kse = w[0] * ke + w[1] * ko1 + w[2] * ke1 + w[3] * ko2
            kso = w[0] * ko + w[1] * ke + w[2] * ko1 + w[3] * ke1
            kv = _gate(_pk(kse * _unpk(vw, 0), kso * _unpk(vw, 1)), dep)
            u = _dot(pltpu.bitcast(fwd_ref[a % 4], bf16), pltpu.bitcast(kv, bf16))
            for p in range(C // 8):
                re = u[16 * p:16 * p + 8]
                im = u[16 * p + 8:16 * p + 16]
                sp_nxt[0, a0 + a, 8 * p:8 * p + 8, :] = im + re
                sp_nxt[1, a0 + a, 8 * p:8 * p + 8, :] = re
                sp_nxt[2, a0 + a, 8 * p:8 * p + 8, :] = im
            fin.append(pltpu.bitcast(im, u32))

        prev = {}

        def pgroup(p, g, dep):
            rows = pl.ds(pl.multiple_of(p * 8 + zsc[g] * 8, 8), 8)
            outs = range(g * PG, (g + 1) * PG)
            acc, hw = {}, {}
            for j in range((g + 1) * PG):
                uu = [sp_cur[k, j, rows, :] for k in range(3)]
                if j == 0 and dep is not None:
                    uu = [pltpu.bitcast(_gate(pltpu.bitcast(x, u32), dep), f32) for x in uu]
                for a in outs:
                    l = a - j
                    if l < 0:
                        continue
                    if l not in hw:
                        hw[l] = [sp_cur[3 + k, l, rows, :] for k in range(3)]
                    for k in range(3):
                        pr = hw[l][k] * uu[k]
                        acc[a, k] = pr if (a, k) not in acc else acc[a, k] + pr
            d = None
            for a in outs:
                re = acc[a, 0] - acc[a, 2]
                im = acc[a, 0] + acc[a, 1]
                if a == 0:
                    wr, wi = re, im
                else:
                    wr, wi = re + prev[p][0], im + prev[p][1]
                prev[p] = (re, im)
                pk = pltpu.bitcast(pltpu.pack_elementwise([wr, wi], packed_dtype=bf16), u32)
                ws_cur[a, p * 8:p * 8 + 8, :] = pk
                if a % 2 == 1:
                    d = pk if d is None else d | pk
            return d & zmask

        dots = []
        for a in chunks:
            if do_fwd:
                dots += [(uf, a), (hf, a)]
            if do_inv:
                dots += [(inv, a)]
            for cw in pre:
                dots += [(lambda it, dep, cw=cw: win_presum(cw, it, dep), it)
                         for it in range(a * 28 // NC, (a + 1) * 28 // NC)]
        cost = [PC if fn not in (uf, hf, inv) else 256 for fn, _ in dots]
        pos = (np.cumsum(cost) - cost - LEAD * 256) / sum(cost) * STR
        nd = len(dots)
        if not do_prod:
            for fn, a in dots:
                fn(a, None)
            return
        ng = NC // PG
        order = [(p, g) for p in range(C // 8) for g in range(ng)]
        if own:
            order = [x for x in order if x[1] < ng - 1] + [x for x in order if x[1] == ng - 1]
        wts = [sum(a + 1 for a in range(g * PG, (g + 1) * PG)) for _, g in order]
        cum = np.cumsum(wts) / sum(wts)
        if own:
            ca = cum[(C // 8) * (ng - 1) - 1]
            n = NC - PG
            dots += [(lambda a, dep: inv(a, dep, True), a) for a in range(n)]
            pos = list(pos * ca / STR) + [ca + k * (OS - ca) / n for k in range(n)]
            nd = len(dots)
        i0 = 0 if mid is None else P0 * ng
        base = 0.0 if i0 == 0 else cum[i0 - 1]
        cum = (cum - base) / (1.0 - base)
        d = 0
        dep = None
        i = 0
        for p, g in order:
            if i == i0:
                if mid is not None:
                    mid()
                while d < nd and pos[d] <= 0:
                    dots[d][0](dots[d][1], None)
                    d += 1
            if i == RQ:
                assert d == nd
                dep = dep | (_or_all(fin[-RN:]) & zmask)
            dep = pgroup(p, g, dep)
            while i >= i0 and d < nd and pos[d] <= cum[i]:
                dots[d][0](dots[d][1], dep)
                d += 1
            i += 1

    kf[0:8, :] = jnp.zeros((8, 128), u32)

    with jax.named_scope('conv'):
        def first_body(it, carry):
            wait_all(kvh0_copies(it))

            @pl.when(it == K1)
            def _():
                start_all(kvh_copies(1))
            conv_stage(-1, 1, False, True, False, range(4), it * 4)
            return carry
        jax.lax.fori_loop(0, NC // 4, first_body, 0)
        xb[:, 0:TM, :] = jnp.zeros((NB, TM, 128), f32)
        wait_all(small2)
        inv_ref[2:4] = inv_ref[0:2] ^ sign
        for r in range(S // 128):
            row = bsp_ref[r:r + 1, :].astype(f32)
            bcol[r * 128:(r + 1) * 128, :] = 0.5 * jnp.broadcast_to(row, (128, 128)).T

        def mid0():
            cps = kvh_copies(1)
            wait_all(cps[:2])
            start_all(kvh_copies(2))
            wait_all(cps[2:])
        conv_stage(0, 0, True, True, False, mid=mid0)

        def conv_body(ii, carry):
            for e in range(2):
                c = 2 * ii + 1 + e
                cps = kvh_copies(c + 1)
                if e == 0:
                    @pl.when(c >= 2)
                    def _():
                        wait_all(win_copies(c - 2))
                    wait_all(cps[:2])
                    start_all(kvh_copies(c + 2))
                    start_all(win_copies(c - 1))
                    cw = jnp.where(c >= 2, c - 2, NB - 1)
                else:
                    wait_all(win_copies(c - 2))
                    wait_all(cps[:2])

                    @pl.when(c + 2 < NB)
                    def _():
                        start_all(kvh_copies(c + 2))

                    @pl.when(c + 2 == NB)
                    def _():
                        start_all(win_copies(c))
                        q_copy0.start()
                    start_all(win_copies(c - 1))
                    cw = c - 2
                wait_all(cps[2:])
                conv_stage(c, 1 - e, True, True, True, pre=(cw,))
            return carry
        jax.lax.fori_loop(0, NB // 2 - 1, conv_body, 0)
        wait_all(win_copies(NB - 3))
        start_all(win_copies(NB - 1))
        q_copy0b.start()
        wait_all(win_copies(NB - 2))
        conv_stage(NB - 1, 1, True, False, True, pre=(NB - 3, NB - 2), own=True)

    q_copy0.wait()
    wait_all(win_copies(NB - 1))

    conv_stage(NB, 0, False, False, True, range(NC - PG, NC))
    for it in range(28):
        win_presum(NB - 1, it, None)

    def wout_b(t, lo, hi):
        if t == 1:
            return pltpu.bitcast(wout_raw[0:FQ, lo:hi], u32)
        if t == 4:
            return pltpu.bitcast(wout_raw[FQ:FH, D2 + lo:D2 + hi], u32)
        return wout_s[SUMS.index(t), :, lo:hi]

    RG = 16
    NG = H // RG

    def a_buf(ref):
        return (lambda t: _ld(ref, t, 0, D2)), (lambda t, lo, g, val: _st_eo(ref, t, lo, g * RG, val))

    def prologue_steps(i, src, a_st, groups=range(NG), idst=None):
        for g in groups:
            st = []
            for hh in range(2):
                r = pl.multiple_of(i * TM + hh * H + g * RG, RG)
                rd = r if idst is None else pl.multiple_of(idst * TM + hh * H + g * RG, RG)
                if src is qbuf:
                    xq = pltpu.bitcast(src[pl.ds(r, RG), :], u32)
                    x = jnp.concatenate([_unpk(xq, 0), _unpk(xq, 1)], axis=0)
                else:
                    x = _ld_eo(src, r, 0, NB)
                x1 = x + _ln(x) * _ld_eo(ybuf, r, 0, NB)
                for c in range(NB):
                    xa[c, pl.ds(rd, 8, stride=2), :] = x1[0:8, c * 128:(c + 1) * 128]
                    xa[c, pl.ds(rd + 1, 8, stride=2), :] = x1[8:16, c * 128:(c + 1) * 128]
                m = jnp.mean(x1, axis=-1, keepdims=True)
                xc = x1 - m
                rs = jax.lax.rsqrt(jnp.mean(xc * xc, axis=-1, keepdims=True) + EPS)
                st.append((pl.multiple_of((i if idst is None else idst) * TM + hh * H + g * RG + zsc[1] * RG, RG), m, rs))
                yield _stat_dep(rs) & zmask
            for (lo, hi) in _chunks(D2, PW):
                q4 = []
                for hh in range(2):
                    rw, m, rs = st[hh]
                    for o in (0, D2):
                        q4.append((_ld_eo(xa, rw, (o + lo) // 128, (o + hi) // 128) - m) * rs)
                ops = _a_ops(*q4)
                yield _or_all([a_st(t, lo, g, ops[t]) for t in range(7)]) & zmask

    def prologue0(a_st):
        def row(j, k):
            return pl.multiple_of(j * RG + zsc[k] * RG, RG)

        def ldq(j, k):
            xq = pltpu.bitcast(qbuf[pl.ds(row(j, k), RG), :], u32)
            return jnp.concatenate([_unpk(xq, 0), _unpk(xq, 1)], axis=0)

        def rstd(xc):
            return jax.lax.rsqrt(jnp.mean(xc * xc, axis=-1, keepdims=True) + EPS)
        js = range(2 * NG)
        m1 = [jnp.mean(ldq(j, 0), axis=-1, keepdims=True) for j in js]
        r1 = [rstd(ldq(j, 1) - m1[j]) for j in js]
        m2 = []
        for j in js:
            x = ldq(j, 2)
            x1 = x + (x - m1[j]) * r1[j] * _ld_eo(ybuf, j * RG, 0, NB)
            for c in range(NB):
                xa[c, pl.ds(j * RG, 8, stride=2), :] = x1[0:8, c * 128:(c + 1) * 128]
                xa[c, pl.ds(j * RG + 1, 8, stride=2), :] = x1[8:16, c * 128:(c + 1) * 128]
            m2.append(jnp.mean(x1, axis=-1, keepdims=True))
        r2 = [rstd(_ld_eo(xa, row(j, 0), 0, NB) - m2[j]) for j in js]
        for g in range(NG):
            for (lo, hi) in _chunks(D2, PW):
                q4 = [(_ld_eo(xa, row(j, 1), (o + lo) // 128, (o + hi) // 128) - m2[j]) * r2[j]
                      for j in (g, NG + g) for o in (0, D2)]
                ops = _a_ops(*q4)
                for t in range(7):
                    a_st(t, lo, g, ops[t])

    PS = 2 + len(_chunks(D2, PW))

    def z2_steps(i, fence):
        for g in range(NG):
            rq = pl.multiple_of(i * H + g * RG, RG)
            fence()
            st = []
            for hh in range(2):
                def row(k):
                    return pl.multiple_of(hh * H + g * RG + zsc[k] * RG, RG)
                m = jnp.mean(_ld_eo(zs, row(0), 0, FH // 128), axis=-1, keepdims=True)
                xc = _ld_eo(zs, row(1), 0, FH // 128) - m
                v = jnp.mean(xc * xc, axis=-1, keepdims=True)
                st.append((row(2), m, 0.5 * jax.lax.rsqrt(v + 4.0 * EPS)))
            yield (_stat_dep(st[0][2]) | _stat_dep(st[1][2])) & zmask
            for (lo, hi) in _chunks(FQ, ZW):
                q4 = []
                for hh in range(2):
                    rw, m, rs = st[hh]
                    for o in (0, FQ):
                        q4.append((_ld_eo(zs, rw, (o + lo) // 128, (o + hi) // 128) - m) * rs)
                ops = _b_ops(*q4)
                yield _or_all([_st_eo(z2ops, t, lo, rq, ops[t]) for t in range(7)]) & zmask

    def spread(nsteps, first, last, sl):
        lo, hi = first * sl, (last + 1) * sl - 1
        return [lo + (k * (hi - lo)) // max(nsteps - 1, 1) for k in range(nsteps)]

    def anchors(steps, slots):
        state = [0]

        def take(n):
            deps = []
            for _ in range(n):
                d = None
                while slots and slots[0] <= state[0]:
                    slots.pop(0)
                    dn = next(steps)
                    d = dn if d is None else d | dn
                deps.append(d)
                state[0] += 1
            return deps
        return take

    def wout_steps():
        for g in range(FQ // WRB):
            for (lo, hi) in _chunks(D2, WC):
                raw = [pltpu.bitcast(wout_raw[r0 + g * WRB:r0 + (g + 1) * WRB, c0 + lo:c0 + hi], u32)
                       for r0 in (0, FQ) for c0 in (0, D2)]
                ev = _b_ops(*[_unpk(x, 0) for x in raw])
                od = _b_ops(*[_unpk(x, 1) for x in raw])
                pks = [_pk(ev[t], od[t]) for t in SUMS]
                for k in range(5):
                    wout_s[k, g * WRB // 2:(g + 1) * WRB // 2, lo:hi] = pks[k]
                yield _or_all(pks) & zmask

    def mm1(i, a_ld, psteps, nps):
        hist = []

        def fence():
            if len(hist) >= ZK:
                zs[FH // 128 + zsc[0], 0:8, :] = hist[-ZK][0:8, 0:128]

        def half(off, steps, slots, store):
            take = anchors(steps, slots)
            for (lo, hi) in _chunks(FQ, TN):
                m = []
                for t in range(7):
                    deps = take((hi - lo) // 128 * SL1)
                    m.append(_dot(a_ld(t), _gate_cols(win_s[t, :, off + lo:off + hi], deps)))
                    hist.append(m[-1])
                c11, c12, c21, c22 = _c_blocks(m)
                store(0, lo, hi, _gelu(c11))
                store(0, FQ + lo, FQ + hi, _gelu(c12))
                store(1, lo, hi, _gelu(c21))
                store(1, FQ + lo, FQ + hi, _gelu(c22))

        def store_z2(hh, lo, hi, val):
            for c in range(lo // 128, hi // 128):
                zs[c, hh * H:(hh + 1) * H, :] = val[:, c * 128 - lo:(c + 1) * 128 - lo]

        def store_z1(hh, lo, hi, val):
            z1buf[pl.ds(pl.multiple_of(i * H + hh * (H // 2), H // 2), H // 2), lo:hi] = _pk(val[:H // 2], val[H // 2:])

        half(FQ, psteps, spread(nps, PA[0], PA[1], SL1), store_z2)
        del hist[:]
        half(0, z2_steps(i, fence), spread(NG * (1 + len(_chunks(FQ, ZW))), ZA[0], ZA[1], SL1), store_z1)

    def ws_steps(i, ws_ref):
        G = BG
        for g in range(H // G):
            r1 = pl.ds(pl.multiple_of(i * TM + g * G, G), G)
            r2 = pl.ds(pl.multiple_of(i * TM + H + g * G, G), G)
            for t in range(NT):
                raw = [pltpu.bitcast(wsp_raw[rr, c0:c0 + H], u32)
                       for rr in (r1, r2) for c0 in (t * TM, t * TM + H)]
                ev = _a_ops(*[_unpk(x, 0) for x in raw])
                od = _a_ops(*[_unpk(x, 1) for x in raw])
                vals = [raw[0] if u == 2 else raw[3] if u == 3 else _pk(ev[u], od[u]) for u in range(7)]
                for u in range(7):
                    ws_ref[u + zsc[0], g * G // 2:(g + 1) * G // 2, t * H:(t + 1) * H] = vals[u]
                yield _or_all([vals[u] for u in (0, 1, 4, 5, 6)]) & zmask

    def mm23(i, inext, ws_ref, src, store, take, done=None):
        r = pl.multiple_of(i * TM, TM)
        for (lo, hi) in _chunks(FQ, TN):
            wdt = hi - lo
            m = [_dot(_ld(ws_ref, t, 0, S // 2), _gate_cols(z2ops[t, :, lo:hi], take(wdt // 128 * SL2)))
                 for t in range(7)]
            c11, c12, c21, c22 = _c_blocks(m)
            b1 = jnp.concatenate([bcol[pl.ds(r, H), :]] * (wdt // 128), axis=1)
            b2 = jnp.concatenate([bcol[pl.ds(r + H, H), :]] * (wdt // 128), axis=1)
            def z1(hh, c0):
                w = z1buf[pl.ds(pl.multiple_of(i * H + hh * (H // 2), H // 2), H // 2), c0:c0 + wdt]
                return jnp.concatenate([_unpk(w, 0), _unpk(w, 1)], axis=0)
            p11 = z1(0, lo) * (c11 + b1)
            p12 = z1(0, FQ + lo) * (c12 + b1)
            p21 = z1(1, lo) * (c21 + b2)
            p22 = z1(1, FQ + lo) * (c22 + b2)
            ops = _a_ops(p11, p12, p21, p22)
            for t in range(7):
                _st(pa, t, lo, 0, ops[t].astype(bf16))
        take3 = anchors(ws_steps(inext, ws_ref), spread(H // BG * NT, BA[0], BA[1], SL3))
        for (lo, hi) in _chunks(D2, TN):
            m = [_dot(_ld(pa, t, 0, FQ), _gate_cols(wout_b(t, lo, hi), take3((hi - lo) // 128 * SL3)))
                 for t in range(7)]
            c11, c12, c21, c22 = _c_blocks(m)
            def res(hh, c0):
                return jnp.concatenate([src[c, pl.ds(r + hh * H, H), :]
                                        for c in range(c0 // 128, (c0 + hi - lo) // 128)], axis=1)
            store(0, lo, hi, res(0, lo) + c11)
            store(0, D2 + lo, D2 + hi, res(0, D2 + lo) + c12)
            store(1, lo, hi, res(1, lo) + c21)
            store(1, D2 + lo, D2 + hi, res(1, D2 + lo) + c22)
            if done is not None:
                done(lo)

    def out_copy(i, slot, los=range(0, D2, TN)):
        rows = pl.ds(pl.multiple_of(i * TM, TM), TM)
        return [pltpu.make_async_copy(obuf.at[slot, :, c0:c0 + TN], out_hbm.at[rows, c0:c0 + TN], sem_out.at[slot])
                for lo in los for c0 in (lo, D2 + lo)]

    def merge(steps_a, slots_a, steps_b, slots_b):
        order = sorted([(q, 0) for q in slots_a] + [(q, 1) for q in slots_b])

        def gen():
            for _, w in order:
                yield next(steps_b if w else steps_a)
        return anchors(gen(), [q for q, _ in order])

    (ld0, st0), (ld1, st1) = a_buf(a0), a_buf(a1)
    prologue0(st0)
    q_copy1.start()
    q_copy0b.wait()

    for layer in range(2):
        def p1_body(ii, carry, layer=layer):
            i = 2 * ii
            if layer == 0:
                @pl.when(ii == 1)
                def _():
                    q_copy1.wait()
                    wout_copy.start()
                    wsp_copy.start()
            src = qbuf if layer == 0 else xb
            mm1(i, ld0, prologue_steps(i + 1, src, st1), NG * PS)
            mm1(i + 1, ld1, prologue_steps(jnp.minimum(i + 2, NT - 1), src, st0), NG * PS)
            return carry

        with jax.named_scope(f'p1_{layer}'):
            jax.lax.fori_loop(0, NT // 2, p1_body, 0)

        if layer == 0:
            wout_copy.wait()
            wsp_copy.wait()
            for _ in ws_steps(0, ws0):
                pass

        if layer == 0:
            def p2_body(i, carry):
                r = pl.multiple_of(i * TM, TM)

                def store(hh, lo, hi, val):
                    for c in range(lo // 128, hi // 128):
                        xb[c, pl.ds(r + hh * H, H), :] = val[:, c * 128 - lo:(c + 1) * 128 - lo]
                g0 = 2 * jnp.clip(i - 1, 0, NG // 2 - 1)
                take = merge(wout_steps(), spread(FQ // WRB * (D2 // WC), WA[0], WA[1], SL2),
                             prologue_steps(0, xb, st0, (g0, g0 + 1), jnp.where(i == 0, NT, 0)),
                             spread(2 * PS, QA[0], QA[1], SL2))
                mm23(i, (i + 1) % NT, ws0, xa, store, take)
                return carry
            with jax.named_scope(f'p2_{layer}'):
                jax.lax.fori_loop(0, NT, p2_body, 0)
        else:
            def p2_body(i, carry):
                slot = i % 2

                def store(hh, lo, hi, val):
                    obuf[slot, hh * H:(hh + 1) * H, lo:hi] = val.astype(bf16)

                @pl.when(i >= 2)
                def _():
                    wait_all(out_copy(i - 2, slot))
                mm23(i, (i + 1) % NT, ws0, xa, store, anchors(None, []),
                     lambda lo: start_all(out_copy(i, slot, (lo,))))
                return carry
            with jax.named_scope(f'p2_{layer}'):
                jax.lax.fori_loop(0, NT, p2_body, 0)
            wait_all(out_copy(NT - 2, 0))
            wait_all(out_copy(NT - 1, 1))


@jax.jit
def pallas_interleave_layers__ssm_conv_h3__mixer_gmlp__prompt_kernel(
    A_q: jax.Array,
    A_k: jax.Array,
    A_v: jax.Array,
    A_shift_k: jax.Array,
    A_ssm_k: jax.Array,
    A_ssm_D: jax.Array,
    B_x: jax.Array,
    B_w_in: jax.Array,
    B_w_sp: jax.Array,
    B_b_sp: jax.Array,
    B_w_out: jax.Array,
):
    fwd_np, inv_np = _dft_mats()
    fwd = jnp.asarray(fwd_np)
    inv = jnp.asarray(inv_np)
    zero = jnp.asarray(np.zeros((8,), np.int32))

    any_spec = pl.BlockSpec(memory_space=pl.ANY)
    smem_spec = pl.BlockSpec(memory_space=pltpu.SMEM)

    scratch = [
        pltpu.VMEM((NB, S, 128), bf16),
        pltpu.VMEM((NB, S, 128), bf16),
        pltpu.VMEM((NB, 128, S), bf16),
        pltpu.VMEM((S, D), bf16),
        pltpu.VMEM((D, F), bf16),
        pltpu.VMEM((7, D2 // 2, FH), u32),
        pltpu.VMEM((S, S), bf16),
        pltpu.VMEM((FH, D), bf16),
        pltpu.VMEM((5, FQ // 2, D2), u32),
        pltpu.VMEM((NB, S + 16, 128), f32),
        pltpu.VMEM((NB, S + TM + 16, 128), f32),
        pltpu.VMEM((NB, S + 16, 128), f32),
        pltpu.VMEM((S // 2, FH), u32),
        pltpu.VMEM((7, S // 4, FQ), u32),
        pltpu.VMEM((FH // 128 + 2, TM + 16, 128), f32),
        pltpu.VMEM((7, H // 2, D2), u32),
        pltpu.VMEM((7, H // 2, D2), u32),
        pltpu.VMEM((7, H // 2, S // 2), u32),
        pltpu.VMEM((7, H // 2, FQ), u32),
        pltpu.VMEM((S, 128), f32),
        pltpu.VMEM((2, TM, D), bf16),
        pltpu.VMEM((S // 2 + 8, 128), u32),
        pltpu.VMEM((6, NC + 1, CP, 128), f32),
        pltpu.VMEM((6, NC + 1, CP, 128), f32),
        pltpu.VMEM((NC, C, 128), u32),
        pltpu.VMEM((NC, C, 128), u32),
        pltpu.VMEM((NB, 8, 128), f32),
        pltpu.VMEM((KS, D), bf16),
        pltpu.VMEM((NB, 128), bf16),
        pltpu.VMEM((S // 128, 128), bf16),
        pltpu.VMEM((4, C, C), u32),
        pltpu.VMEM((4, C // 2, 2 * C), u32),
        pltpu.SemaphoreType.DMA((NB,)),
        pltpu.SemaphoreType.DMA((NB,)),
        pltpu.SemaphoreType.DMA((5,)),
        pltpu.SemaphoreType.DMA((2,)),
        pltpu.SemaphoreType.DMA((4,)),
        pltpu.SemaphoreType.DMA((3,)),
    ]

    out = pl.pallas_call(
        _kernel,
        in_specs=[smem_spec] + [any_spec] * 12,
        out_specs=any_spec,
        out_shape=jax.ShapeDtypeStruct((S, D), bf16),
        scratch_shapes=scratch,
        compiler_params=pltpu.CompilerParams(vmem_limit_bytes=127 * 1024 * 1024, disable_bounds_checks=True),
    )(
        zero,
        A_q.reshape(S, D), A_k.reshape(S, D), A_v.reshape(S, D),
        A_shift_k.T, A_ssm_k.reshape(NB, 128, S), A_ssm_D.reshape(NB, 128),
        B_w_in, B_w_sp, B_b_sp.reshape(S // 128, 128), B_w_out,
        fwd, inv,
    )
    return out.reshape(1, S, D)
```
